```python
import jax
import jax.numpy as jnp

def _softmax(x, axis=-1):
    return jax.nn.softmax(x, axis=axis)

def _gelu(x):
    return jax.nn.gelu(x, approximate=True)

def _silu(x):
    return jax.nn.silu(x)

def _sigmoid(x):
    return jax.nn.sigmoid(x)

def _layernorm(x, axis=-1, eps=1e-05):
    m = jnp.mean(x, axis=axis, keepdims=True)
    v = jnp.var(x, axis=axis, keepdims=True)
    return (x - m) / jnp.sqrt(v + eps)

def _scatter_add(tgt, idx, src, axis=0):
    return tgt.at[idx].add(src)

def _segment_sum(src, seg, n):
    return jax.ops.segment_sum(src, seg, n)

class _Rng:

    def __init__(self, key):
        self._k = key

    def _next(self):
        self._k, sub = jax.random.split(self._k)
        return sub

    def normal(self, shape):
        return jax.random.normal(self._next(), shape, dtype=jnp.bfloat16)

    def randint(self, lo, hi, shape):
        return jax.random.randint(self._next(), shape, lo, hi, dtype=jnp.int32)

    def uniform(self, shape, lo=0.0, hi=1.0):
        return jax.random.uniform(self._next(), shape, jnp.bfloat16, lo, hi)

    def permutation(self, n):
        return jax.random.permutation(self._next(), n)
kernel_name = 'adaLN_cond__compressed_kv_cla__mixer_s_mlp__prompt'

def setup_inputs():
    _rng = _Rng(jax.random.key(int.from_bytes(__import__("os").urandom(4), "little")))
    _w = lambda a: (lambda t: t.astype(jnp.bfloat16) if jnp.issubdtype(t.dtype, jnp.floating) else t)(jnp.asarray(a))

    def _A_setup():
        B, H, Sq, Sk, D, M = (1, 32, 2048, 2048, 128, 640)
        Dc = 4 * D
        return {'x': _w((lambda *s: _rng.normal(s) * 0.05)(B, Sq, M)), 'c_kv': _w((lambda *s: _rng.normal(s) * 0.05)(B, Sk, Dc)), 'w_q': _w((lambda *s: _rng.normal(s) * 0.05)(M, H, D) * M ** (-0.5)), 'w_uk': _w((lambda *s: _rng.normal(s) * 0.05)(Dc, H, D) * Dc ** (-0.5)), 'w_uv': _w((lambda *s: _rng.normal(s) * 0.05)(Dc, H, D) * Dc ** (-0.5)), 'w_o': _w((lambda *s: _rng.normal(s) * 0.05)(H, D, M) * (H * D) ** (-0.5))}
    _A_in = _A_setup()

    def _B_setup():
        B, S, D, F = (1, 2048, 640, 1728)
        return {'x': _w((lambda *s: _rng.normal(s) * 0.05)(B, S, D)), 'w1': _w((lambda *s: _rng.normal(s) * 0.05)(D, D) * D ** (-0.5)), 'w2': _w((lambda *s: _rng.normal(s) * 0.05)(D, D) * D ** (-0.5)), 'w3': _w((lambda *s: _rng.normal(s) * 0.05)(D, F) * D ** (-0.5)), 'w4': _w((lambda *s: _rng.normal(s) * 0.05)(F, D) * F ** (-0.5))}
    _B_in = _B_setup()
    return {'A_x': _A_in['x'], 'A_c_kv': _A_in['c_kv'], 'A_w_q': _A_in['w_q'], 'A_w_uk': _A_in['w_uk'], 'A_w_uv': _A_in['w_uv'], 'A_w_o': _A_in['w_o'], 'B_x': _B_in['x'], 'B_w1': _B_in['w1'], 'B_w2': _B_in['w2'], 'B_w3': _B_in['w3'], 'B_w4': _B_in['w4'], 'c': _w((lambda *s: _rng.normal(s) * 0.05)(1, 640)), 'w_mod': _w((lambda *s: _rng.normal(s) * 0.05)(640, 6 * 640) * 640 ** (-0.5))}

def reference(A_x, A_c_kv, A_w_q, A_w_uk, A_w_uv, A_w_o, B_x, B_w1, B_w2, B_w3, B_w4, c, w_mod):

    def _A_ref(x, c_kv, w_q, w_uk, w_uv, w_o):
        B, Sq, M = (x.shape[0], x.shape[1], x.shape[2])
        Sk = c_kv.shape[1]
        H, D = (w_q.shape[1], w_q.shape[2])
        q = jnp.einsum('bqm,mhd->bhqd', x, w_q)
        k = jnp.einsum('bkc,chd->bhkd', c_kv, w_uk)
        v = jnp.einsum('bkc,chd->bhkd', c_kv, w_uv)
        scores = jnp.einsum('bhqd,bhkd->bhqk', q, k) * D ** (-0.5)
        off = Sk - Sq
        qi = jnp.arange(Sq)[:, None]
        kj = jnp.arange(Sk)[None, :]
        cmask = kj <= qi + off
        scores = jnp.where(cmask[None, None], scores, -1000000000.0)
        p = _softmax(scores, axis=-1)
        ctx = jnp.einsum('bhqk,bhkd->bhqd', p, v)
        return jnp.einsum('bhqd,hdm->bqm', ctx, w_o)

    def _B_ref(x, w1, w2, w3, w4):
        B, S, D = x.shape
        h = _gelu(_layernorm(x, axis=-1) @ w1)
        c = D // 4
        g0 = jnp.pad(h[:, :, 0 * c:1 * c], ((0, 0), (1, 0), (0, 0)))[:, :S, :]
        g1 = jnp.pad(h[:, :, 1 * c:2 * c], ((0, 0), (0, 1), (0, 0)))[:, 1:, :]
        g2 = jnp.pad(h[:, :, 2 * c:3 * c], ((0, 0), (2, 0), (0, 0)))[:, :S, :]
        g3 = jnp.pad(h[:, :, 3 * c:], ((0, 0), (0, 2), (0, 0)))[:, 2:, :]
        hs = jnp.concatenate([g0, g1, g2, g3], axis=-1) @ w2
        x1 = x + hs
        h2 = _gelu(_layernorm(x1, axis=-1) @ w3) @ w4
        return x1 + h2
    x = A_x
    mod = (_silu(c) @ w_mod).reshape(c.shape[0], 6, 1, -1)
    sa, ca, ga, sb, cb, gb = (mod[:, 0].copy(), mod[:, 1].copy(), mod[:, 2].copy(), mod[:, 3].copy(), mod[:, 4].copy(), mod[:, 5].copy())
    h = _layernorm(x, axis=-1) * (1 + ca) + sa
    x = x + ga * _A_ref(h, A_c_kv, A_w_q, A_w_uk, A_w_uv, A_w_o)
    h = _layernorm(x, axis=-1) * (1 + cb) + sb
    x = x + gb * _B_ref(h, B_w1, B_w2, B_w3, B_w4)
    return x
```

```python
import functools
import jax
import jax.numpy as jnp
from jax import lax
import jax.experimental.pallas as pl
import jax.experimental.pallas.tpu as pltpu

F32 = jnp.float32
BF16 = jnp.bfloat16
U32 = jnp.uint32
LOG2E = 1.4426950408889634
NEG = -1e9 * LOG2E


def _dot(a, b):
    return jnp.dot(a, b, preferred_element_type=F32)


def _dot_nt(a, b):
    return lax.dot_general(a, b, (((1,), (1,)), ((), ())), preferred_element_type=F32)


def _ln(x):
    m = jnp.mean(x, axis=-1, keepdims=True)
    xc = x - m
    v = jnp.mean(xc * xc, axis=-1, keepdims=True)
    return xc * lax.rsqrt(v + 1e-5)


def _gelu(x):
    return jax.nn.gelu(x, approximate=True)


def make(nh=32, lag=2, pchunk=512, pstart=7, RC=256, border=0, peel=True, finpos=0):
    S, M, C, H, D, F = 2048, 640, 512, 32, 128, 1728
    BQ = 256
    NQ = S // BQ
    G = 16

    def kernel(x_hbm, ckv_hbm, wq_hbm, wuk_hbm, wuv_hbm, wo_hbm, w1_hbm, w2_hbm, w3_hbm, w4_hbm, c_hbm, wmod_hbm,
               o_hbm,
               x_v, ckv_v, wq_r, wuk_r, wuv_r, wo_v, w1_v, w2_v, w3_v, w4_v, c_v, wma_v, wmb_v,
               wq_s, wk_s, wv_s, mod_v, h_v, q_v, k_v, v_v, acc_v, g_v, o_v, sems, never_ref):
        never_ref[0] = pl.program_id(0) - 5
        NG = H // G
        PG = G // 2

        def cp(i, src, dst):
            return pltpu.make_async_copy(src, dst, sems.at[i])

        def wcp(i, hbm, raw, g):
            return cp(i, hbm.bitcast(U32).at[:, pl.ds(PG * g, PG), :], raw.at[g])

        d_ckv = cp(0, ckv_hbm, ckv_v)
        d_uk = [wcp(1 + g, wuk_hbm, wuk_r, g) for g in range(NG)]
        d_uv = [wcp(3 + g, wuv_hbm, wuv_r, g) for g in range(NG)]
        d_q = [wcp(5 + g, wq_hbm, wq_r, g) for g in range(NG)]
        d_c = cp(7, c_hbm, c_v)
        d_ma = cp(8, wmod_hbm.at[:, pl.ds(0, 2 * M)], wma_v)
        d_mb = cp(9, wmod_hbm.at[:, pl.ds(2 * M, 4 * M)], wmb_v)
        d_x = cp(10, x_hbm, x_v)
        d_wo = [cp(11 + g, wo_hbm.at[pl.ds(G * g, G)], wo_v.at[pl.ds(G * g, G)]) for g in range(NG)]
        d_w = [cp(13, w1_hbm, w1_v), cp(14, w2_hbm, w2_v), cp(15, w3_hbm, w3_v), cp(16, w4_hbm, w4_v)]
        SEM_O = 17

        def extract(raw, g, dst, n):
            r2 = raw.at[g].reshape(n * PG, D)
            for j in range(PG):
                b = r2[pl.ds(j, n, stride=PG), :]
                dst[G * g + 2 * j] = pltpu.bitcast(b << U32(16), F32).astype(BF16)
                dst[G * g + 2 * j + 1] = pltpu.bitcast(b & U32(0xFFFF0000), F32).astype(BF16)

        qscale = (D ** -0.5) * LOG2E

        def proj_q(hd, r, n):
            rows = pl.ds(r, n)
            q_v[rows, :] = (_dot(h_v[rows, :], wq_s[hd]) * qscale).astype(BF16)

        def proj_k(hd, r, n):
            rows = pl.ds(r, n)
            k_v[rows, :] = _dot(ckv_v[rows, :], wk_s[hd]).astype(BF16)

        def proj_v(hd, r, n):
            rows = pl.ds(r, n)
            v_v[rows, :] = _dot(ckv_v[rows, :], wv_s[hd]).astype(BF16)

        def modrow(i):
            return mod_v[0:1, i * M:(i + 1) * M]

        for d in (d_ckv, d_uk[0], d_uv[0], d_c, d_ma, d_x, d_q[0], d_wo[0]):
            d.start()
        d_ckv.wait(); d_uk[0].wait()
        extract(wuk_r, 0, wk_s, C)
        for r in range(0, S, 512):
            proj_k(0, r, 512)
        d_uv[0].wait()
        extract(wuv_r, 0, wv_s, C)
        for r in range(0, S, 512):
            proj_v(0, r, 512)
        d_c.wait(); d_ma.wait()
        cc = c_v[...].astype(F32)
        sc8 = jnp.broadcast_to((cc * jax.nn.sigmoid(cc)).astype(BF16), (8, M))
        mod_v[:, 0:2 * M] = _dot(sc8, wma_v[...])
        d_x.wait()

        def ln_a(r, _):
            rows = pl.ds(pl.multiple_of(r * 256, 256), 256)
            xx = x_v[rows, :].astype(F32)
            h_v[rows, :] = (_ln(xx) * (1.0 + modrow(1)) + modrow(0)).astype(BF16)
            return 0
        lax.fori_loop(0, S // 256, ln_a, 0)
        d_q[0].wait()
        for d in (d_uk[1], d_uv[1], d_q[1], d_wo[1], d_mb, *d_w):
            d.start()
        extract(wq_r, 0, wq_s, M)
        for r in range(0, S, 512):
            proj_q(0, r, 512)
        d_wo[0].wait()

        nv = lax.broadcasted_iota(jnp.int32, (BQ, 128), 1) < never_ref[0]
        tri = (lax.broadcasted_iota(jnp.int32, (128, 128), 1) <= lax.broadcasted_iota(jnp.int32, (128, 128), 0))

        def attention(hd, first, fillers_qk, fillers_v, tail):
            wo_h = wo_v[hd]
            st = {}
            hist = []

            def qk(qi, t):
                d = st.setdefault(qi, dict(ss={}, mp=None, lp=None, acc=None))
                q = q_v[pl.ds(qi * BQ, BQ), :]
                if t < qi:
                    s = _dot_nt(q, k_v[pl.ds(t * 256, 256), :])
                    d['ss'][t] = s
                    x = jnp.maximum(s[:, :128], s[:, 128:])
                else:
                    s0 = _dot_nt(q, k_v[pl.ds(t * 256, 128), :])
                    s1 = _dot_nt(q[128:], k_v[pl.ds(t * 256 + 128, 128), :])
                    s0 = jnp.concatenate([jnp.where(tri, s0[:128], NEG), s0[128:]], axis=0)
                    s1 = jnp.where(tri, s1, NEG)
                    d['ss'][t] = (s0, s1)
                    x = jnp.concatenate([s0[:128], jnp.maximum(s0[128:], s1)], axis=0)
                d['mp'] = x if d['mp'] is None else jnp.maximum(d['mp'], x)

            def fin_max(qi):
                m = jnp.max(st[qi]['mp'], axis=-1, keepdims=True)
                st[qi]['m'] = jnp.broadcast_to(m, (BQ, 128))

            def pv(qi, t):
                d = st[qi]
                mm = d['m']
                if len(hist) >= lag:
                    mm = jnp.where(nv, hist[-lag], mm)
                if t < qi:
                    s = d['ss'][t]
                    p = jnp.exp2(s - jnp.concatenate([mm, mm], axis=1))
                    o = _dot(p.astype(BF16), v_v[pl.ds(t * 256, 256), :])
                    x = p[:, :128] + p[:, 128:]
                else:
                    s0, s1 = d['ss'][t]
                    p0 = jnp.exp2(s0 - mm)
                    p1 = jnp.exp2(s1 - mm[128:])
                    o0 = _dot(p0.astype(BF16), v_v[pl.ds(t * 256, 128), :])
                    o1 = _dot(p1.astype(BF16), v_v[pl.ds(t * 256 + 128, 128), :])
                    o = jnp.concatenate([o0[:128], o0[128:] + o1], axis=0)
                    x = jnp.concatenate([p0[:128], p0[128:] + p1], axis=0)
                hist.append(o)
                d['lp'] = x if d['lp'] is None else d['lp'] + x
                d['acc'] = o if d['acc'] is None else d['acc'] + o

            def fin(qi):
                d = st.pop(qi)
                l = jnp.sum(d['lp'], axis=-1, keepdims=True)
                ctx = (d['acc'] / l).astype(BF16)
                contrib = _dot(ctx, wo_h)
                rows = pl.ds(qi * BQ, BQ)
                if first is True:
                    acc_v[rows, :] = contrib
                elif first is False:
                    acc_v[rows, :] += contrib
                else:
                    acc_v[rows, :] = contrib + jnp.where(first, 0.0, acc_v[rows, :])

            fq = list(fillers_qk)
            qk(0, 0)
            fin_max(0)
            for qi in range(NQ):
                nxt = qi + 1 if qi + 1 < NQ else None
                a = qi + 1
                b = qi + 2 if nxt is not None else 0
                for t in range(max(a, b)):
                    if t < b:
                        qk(nxt, t)
                        if t == b - 1:
                            fin_max(nxt)
                    elif nxt is None and fq:
                        fq.pop(0)()
                    if t < a:
                        pv(qi, t)
                if nxt is None:
                    for _ in range(finpos):
                        if fq:
                            fq.pop(0)()
                fin(qi)
                if tail is not None:
                    tail(qi)
            for f in fq:
                f()
            for f in fillers_v:
                f()

        def head_body(hd, _):
            fq = [functools.partial(proj_q, hd + 1, r, pchunk) for r in range(0, S, pchunk)]
            fk = [functools.partial(proj_k, hd + 1, r, pchunk) for r in range(0, S, pchunk)]
            fv = [functools.partial(proj_v, hd + 1, r, 512) for r in range(0, S, 512)]
            attention(hd, False, fq + fk, fv, None)
            return 0

        for r in range(0, S, 256):
            acc_v[pl.ds(r, 256), :] = jnp.zeros((256, M), F32)

        if peel:
            lax.fori_loop(0, G - 1, head_body, 0)
            for d in (d_uk[1], d_uv[1], d_q[1], d_wo[1]):
                d.wait()
            extract(wuk_r, 1, wk_s, C)
            extract(wuv_r, 1, wv_s, C)
            extract(wq_r, 1, wq_s, M)
            lax.fori_loop(G - 1, nh - 1, head_body, 0)
        d_mb.wait()
        for d in d_w:
            d.wait()
        mod_v[:, 2 * M:] = _dot(sc8, wmb_v[...])

        G0 = 8
        g_v[pl.ds(0, G0), :] = jnp.zeros((G0, M), F32)
        g_v[pl.ds(S + G0, G0), :] = jnp.zeros((G0, M), F32)

        def b1(r):
            rows = pl.ds(r * RC, RC)
            x1 = x_v[rows, :].astype(F32) + modrow(2) * acc_v[rows, :]
            acc_v[rows, :] = x1
            h2 = _ln(x1) * (1.0 + modrow(4)) + modrow(3)
            h_v[rows, :] = h2.astype(BF16)
            g = _gelu(_dot(_ln(h2).astype(BF16), w1_v[...]))
            g_v[pl.ds(r * RC + G0, RC), :] = g

        outs = []
        c128 = lax.broadcasted_iota(jnp.int32, (RC, 128), 1)

        def b2(r):
            base = r * RC + G0

            def sh(d, lo):
                return g_v[pl.ds(base + d, RC), lo:lo + 128]
            t0 = sh(-1, 0)
            t1 = jnp.where(c128 < 32, sh(-1, 128), sh(1, 128))
            t2 = jnp.where(c128 < 64, sh(1, 256), sh(-2, 256))
            t3 = jnp.where(c128 < 96, sh(-2, 384), sh(2, 384))
            t4 = sh(2, 512)
            gs = jnp.concatenate([t0, t1, t2, t3, t4], axis=1).astype(BF16)
            rows = pl.ds(r * RC, RC)
            x1b = h_v[rows, :].astype(F32) + _dot(gs, w2_v[...])
            u = _gelu(_dot_nt(_ln(x1b).astype(BF16), w3_v[...])).astype(BF16)
            y = x1b + _dot(u, w4_v[...])
            o_v[rows, :] = (acc_v[rows, :] + modrow(5) * y).astype(BF16)
            oc = pltpu.make_async_copy(o_v.at[rows, :], o_hbm.at[rows, :], sems.at[SEM_O + r])
            oc.start()
            outs.append(oc)

        NR = S // RC
        if peel:
            attention(H - 1, False, [], [], None)
        b1(0)
        for r in range(NR):
            if r + 1 < NR:
                b1(r + 1)
            b2(r)
        for oc in outs:
            oc.wait()

    def fn(A_x, A_c_kv, A_w_q, A_w_uk, A_w_uv, A_w_o, B_x, B_w1, B_w2, B_w3, B_w4, c, w_mod):
        x = A_x.reshape(S, M)
        ckv = A_c_kv.reshape(S, C)
        hbm = pl.BlockSpec(memory_space=pltpu.HBM)
        out = pl.pallas_call(
            kernel,
            grid=(1,),
            out_shape=jax.ShapeDtypeStruct((S, M), BF16),
            in_specs=[hbm] * 12,
            out_specs=hbm,
            scratch_shapes=[
                pltpu.VMEM((S, M), BF16), pltpu.VMEM((S, C), BF16),
                pltpu.VMEM((H // G, M, G // 2, D), U32), pltpu.VMEM((H // G, C, G // 2, D), U32),
                pltpu.VMEM((H // G, C, G // 2, D), U32),
                pltpu.VMEM((H, D, M), BF16),
                pltpu.VMEM((M, M), BF16), pltpu.VMEM((M, M), BF16), pltpu.VMEM((F, M), BF16), pltpu.VMEM((F, M), BF16),
                pltpu.VMEM((1, M), BF16), pltpu.VMEM((M, 2 * M), BF16), pltpu.VMEM((M, 4 * M), BF16),
                pltpu.VMEM((H, M, D), BF16), pltpu.VMEM((H, C, D), BF16), pltpu.VMEM((H, C, D), BF16),
                pltpu.VMEM((8, 6 * M), F32),
                pltpu.VMEM((S, M), BF16),
                pltpu.VMEM((S, D), BF16), pltpu.VMEM((S, D), BF16), pltpu.VMEM((S, D), BF16),
                pltpu.VMEM((S, M), F32),
                pltpu.VMEM((S + 16, M), F32),
                pltpu.VMEM((S, M), BF16),
                pltpu.SemaphoreType.DMA((17 + S // RC,)),
                pltpu.SMEM((1,), jnp.int32),
            ],
            compiler_params=pltpu.CompilerParams(vmem_limit_bytes=110 * 1024 * 1024),
        )(x, ckv, A_w_q, A_w_uk, A_w_uv, A_w_o, B_w1, B_w2, B_w3.T, B_w4, c, w_mod)
        return out.reshape(1, S, M)
    return jax.jit(fn)


pallas_adaLN_cond__compressed_kv_cla__mixer_s_mlp__prompt_kernel = make()
```

```python
import functools
import jax
import numpy as np
import jax.numpy as jnp
from jax import lax
import jax.experimental.pallas as pl
import jax.experimental.pallas.tpu as pltpu

F32 = jnp.float32
BF16 = jnp.bfloat16
U32 = jnp.uint32
LOG2E = 1.4426950408889634
NEG = -1e9 * LOG2E


def _dot(a, b):
    return jnp.dot(a, b, preferred_element_type=F32)


def _dot_nt(a, b):
    return lax.dot_general(a, b, (((1,), (1,)), ((), ())), preferred_element_type=F32)


def _ln(x):
    m = jnp.mean(x, axis=-1, keepdims=True)
    xc = x - m
    v = jnp.mean(xc * xc, axis=-1, keepdims=True)
    return xc * lax.rsqrt(v + 1e-5)


def _gelu(x):
    return jax.nn.gelu(x, approximate=True)


def make(nh=32, lag=2, pchunk=512, pstart=7, RC=256, border=0, peel=True, finpos=0, skipB=False, pro=1, stop=0, rot=1536, rotpos=1, pvfirst=1, depm=0, slack=0, finlag=0, bord=2, LA=3, lnpos=0):
    S, M, C, H, D, F = 2048, 640, 512, 32, 128, 1728
    BQ = 256
    NQ = S // BQ
    G = 16

    def kernel(x_hbm, ckv_hbm, wq_hbm, wuk_hbm, wuv_hbm, wo_hbm, w1_hbm, w2_hbm, w3_hbm, w4_hbm, c_hbm, wmod_hbm, never_ref,
               o_hbm,
               x_v, ckv_v, wq_r, wuk_r, wuv_r, wo_v, w1_v, w2_v, w3_v, w4_v, c_v, wma_v, wmb_v,
               wq_s, wk_s, wv_s, mod_v, h_v, q_v, k_v, v_v, k_pre, v_pre, acc_v, g_v, o_v, sems):
        NG = H // G
        NW = max(LA - 1, 1)
        PG = G // 2

        def cp(i, src, dst):
            return pltpu.make_async_copy(src, dst, sems.at[i])

        def wcp(i, hbm, raw, g):
            return cp(i, hbm.bitcast(U32).at[:, pl.ds(PG * g, PG), :], raw.at[g])

        d_ckv = cp(0, ckv_hbm, ckv_v)
        d_uk = [wcp(1 + g, wuk_hbm, wuk_r, g) for g in range(NG)]
        d_uv = [wcp(3 + g, wuv_hbm, wuv_r, g) for g in range(NG)]
        d_q = [wcp(5 + g, wq_hbm, wq_r, g) for g in range(NG)]
        d_c = cp(7, c_hbm, c_v)
        d_ma = cp(8, wmod_hbm.at[:, pl.ds(0, 2 * M)], wma_v)
        d_mb = cp(9, wmod_hbm.at[:, pl.ds(2 * M, 4 * M)], wmb_v)
        d_x = cp(10, x_hbm, x_v)
        d_wo = [cp(11, wo_hbm.at[pl.ds(0, NW)], wo_v.at[pl.ds(0, NW)]),
                cp(12, wo_hbm.at[pl.ds(NW, H - NW)], wo_v.at[pl.ds(NW, H - NW)])]
        d_w = [cp(13, w1_hbm, w1_v), cp(14, w2_hbm, w2_v), cp(15, w3_hbm, w3_v), cp(16, w4_hbm, w4_v)]
        SEM_O = 17

        def extract_pair(raw, g, dst, n, j):
            r2 = raw.at[g].reshape(n * PG, D)
            b = r2[pl.ds(j, n, stride=PG), :]
            dst[G * g + 2 * j] = pltpu.bitcast(b << U32(16), F32).astype(BF16)
            dst[G * g + 2 * j + 1] = pltpu.bitcast(b & U32(0xFFFF0000), F32).astype(BF16)

        def extract(raw, g, dst, n):
            for j in range(PG):
                extract_pair(raw, g, dst, n, j)

        qscale = (D ** -0.5) * LOG2E

        def proj_q(hd, r, n):
            rows = pl.ds(r, n)
            q_v[rows, :] = (_dot(h_v[rows, :], wq_s[hd]) * qscale).astype(BF16)

        def proj_k(hd, r, n, dst=None):
            rows = pl.ds(r, n)
            dst = k_v if dst is None else dst
            dst[rows, :] = _dot(ckv_v[rows, :], wk_s[hd]).astype(BF16)

        def proj_v(hd, r, n, dst=None):
            rows = pl.ds(r, n)
            dst = v_v if dst is None else dst
            dst[rows, :] = _dot(ckv_v[rows, :], wv_s[hd]).astype(BF16)

        def modrow(i):
            return mod_v[0:1, i * M:(i + 1) * M]

        def go(*ds):
            for d in ds:
                d.start()

        def ln_a(r):
            rows = pl.ds(r * 256, 256)
            xx = x_v[rows, :].astype(F32)
            h_v[rows, :] = (_ln(xx) * (1.0 + modrow(1)) + modrow(0)).astype(BF16)
            acc_v[rows, :] = jnp.zeros((256, M), F32)

        def kdst(hd):
            return k_v if hd == LA - 1 else k_pre.at[hd]

        def vdst(hd):
            return v_v if hd == LA - 1 else v_pre.at[hd]

        go(d_ckv, d_uk[0], d_uv[0])
        d_ckv.wait(); d_uk[0].wait()
        go(d_c, d_ma, d_x)
        for hd in range(LA):
            for j in range(8):
                if hd == 0:
                    extract_pair(wuk_r, 0, wk_s, C, j)
                proj_k(hd, j * 256, 256, kdst(hd))
        d_uv[0].wait()
        go(d_q[0], d_wo[0])
        lns = list(range(S // 256))
        for hd in range(LA):
            if hd == min(1, LA - 1):
                if hd == 0:
                    extract(wuv_r, 0, wv_s, C)
                d_c.wait(); d_ma.wait(); d_x.wait()
                cc = c_v[...].astype(F32)
                sc8 = jnp.broadcast_to((cc * jax.nn.sigmoid(cc)).astype(BF16), (8, M))
                mod_v[:, 0:2 * M] = _dot(sc8, wma_v[...])
            for j in range(8 if hd < LA - 1 else (S - rot) // 256):
                if hd == 0 and LA > 1:
                    extract_pair(wuv_r, 0, wv_s, C, j)
                proj_v(hd, j * 256, 256, vdst(hd))
                if hd >= min(1, LA - 1) and lns and (LA <= 2 or j % 2 == 0 or hd > 1):
                    ln_a(lns.pop(0))
        while lns:
            ln_a(lns.pop(0))
        d_q[0].wait()
        rest = (d_uk[1], d_uv[1], d_q[1], d_mb, *d_w)
        go(d_wo[1])
        for j in range(8):
            extract_pair(wq_r, 0, wq_s, M, j)
            proj_q(0, j * 256, 256)
        d_wo[0].wait()
        if LA < 3 or stop:
            d_wo[1].wait()
            go(*rest)

        if stop == 1:
            o_v[...] = h_v[...]
            oc = pltpu.make_async_copy(o_v, o_hbm, sems.at[SEM_O]); oc.start(); oc.wait()
            for d in rest:
                d.wait()
            return
        if stop == 2:
            o_v[...] = h_v[...]
            oc = pltpu.make_async_copy(o_v, o_hbm, sems.at[SEM_O]); oc.start(); oc.wait()
            return
        nv = lax.broadcasted_iota(jnp.int32, (BQ, 128), 1) < never_ref[0]
        tri = (lax.broadcasted_iota(jnp.int32, (128, 128), 1) <= lax.broadcasted_iota(jnp.int32, (128, 128), 0))

        def attention(hd, first, fillers_qk, fillers_v, tail, fillers_head=(), k_v=k_v, v_v=v_v):
            wo_h = wo_v[hd]
            st = {}
            hist = []

            def qk(qi, t):
                d = st.setdefault(qi, dict(ss={}, mp=None, lp=None, acc=None))
                q = q_v[pl.ds(qi * BQ, BQ), :]
                if t < qi:
                    s = _dot_nt(q, k_v[pl.ds(t * 256, 256), :])
                    d['ss'][t] = s
                    x = jnp.maximum(s[:, :128], s[:, 128:])
                else:
                    s0 = _dot_nt(q, k_v[pl.ds(t * 256, 128), :])
                    s1 = _dot_nt(q[128:], k_v[pl.ds(t * 256 + 128, 128), :])
                    s0 = jnp.concatenate([jnp.where(tri, s0[:128], NEG), s0[128:]], axis=0)
                    s1 = jnp.where(tri, s1, NEG)
                    d['ss'][t] = (s0, s1)
                    x = jnp.concatenate([s0[:128], jnp.maximum(s0[128:], s1)], axis=0)
                d['mp'] = x if d['mp'] is None else jnp.maximum(d['mp'], x)

            def fin_max(qi):
                m = jnp.max(st[qi]['mp'], axis=-1, keepdims=True)
                st[qi]['m'] = jnp.broadcast_to(m, (BQ, 128))

            def pv(qi, t):
                d = st[qi]
                mm = d['m']
                if len(hist) >= lag and lag > 0:
                    mm = jnp.where(nv, hist[-lag], mm)
                if depm and len(hist) >= 1:
                    mm = jnp.concatenate([mm[:128], jnp.where(nv[:128], hist[-1][:128], mm[128:])], axis=0)
                if t < qi:
                    s = d['ss'][t]
                    p = jnp.exp2(s - jnp.concatenate([mm, mm], axis=1))
                    o = _dot(p.astype(BF16), v_v[pl.ds(t * 256, 256), :])
                    x = p[:, :128] + p[:, 128:]
                else:
                    s0, s1 = d['ss'][t]
                    p0 = jnp.exp2(s0 - mm)
                    p1 = jnp.exp2(s1 - mm[128:])
                    o0 = _dot(p0.astype(BF16), v_v[pl.ds(t * 256, 128), :])
                    o1 = _dot(p1.astype(BF16), v_v[pl.ds(t * 256 + 128, 128), :])
                    o = jnp.concatenate([o0[:128], o0[128:] + o1], axis=0)
                    x = jnp.concatenate([p0[:128], p0[128:] + p1], axis=0)
                hist.append(o)
                d['lp'] = x if d['lp'] is None else d['lp'] + x
                d['acc'] = o if d['acc'] is None else d['acc'] + o

            def fin(qi):
                d = st.pop(qi)
                l = jnp.sum(d['lp'], axis=-1, keepdims=True)
                ctx = (d['acc'] / l).astype(BF16)
                contrib = _dot(ctx, wo_h)
                rows = pl.ds(qi * BQ, BQ)
                if first is True:
                    acc_v[rows, :] = contrib
                elif first is False:
                    acc_v[rows, :] += contrib
                else:
                    acc_v[rows, :] = contrib + jnp.where(first, 0.0, acc_v[rows, :])

            fq = list(fillers_qk)
            fh = list(fillers_head)
            tiles = [(i, t) for i in range(NQ) for t in range(i + 1)]
            qptr = [0]

            def emit_qk_upto(n):
                any_ = False
                while qptr[0] < min(n, len(tiles)):
                    i, t = tiles[qptr[0]]
                    qk(i, t)
                    if fh:
                        fh.pop(0)()
                    if t == i:
                        fin_max(i)
                    qptr[0] += 1
                    any_ = True
                return any_

            def T(i):
                return i * (i + 1) // 2
            emit_qk_upto(1)
            pend_fin = []
            for (qi, t) in tiles:
                if slack == 0:
                    need = T(qi + 1) + t + 1
                    if t == qi:
                        need = T(qi + 2)
                else:
                    need = T(qi + 1) + -(-((t + 1 + slack) * (qi + 2)) // (qi + 1))
                if not pvfirst:
                    if not emit_qk_upto(need) and qptr[0] >= len(tiles) and fq:
                        fq.pop(0)()
                pv(qi, t)
                if pvfirst:
                    if not emit_qk_upto(need) and qptr[0] >= len(tiles) and fq:
                        fq.pop(0)()
                for e in pend_fin:
                    e[0] -= 1
                while pend_fin and pend_fin[0][0] <= 0:
                    fin(pend_fin.pop(0)[1])
                if t == qi:
                    if finlag == 0 or qi == NQ - 1:
                        while pend_fin:
                            fin(pend_fin.pop(0)[1])
                        if qi == NQ - 1:
                            for _ in range(finpos):
                                if fq:
                                    fq.pop(0)()
                        fin(qi)
                    else:
                        pend_fin.append([finlag, qi])
            for f in fq:
                f()
            for f in fillers_v:
                f()

        def vhead(hd):
            return [functools.partial(proj_v, hd, r, 256) for r in range(S - rot, S, 256)]

        def head_body(hd, _):
            fq = [functools.partial(proj_q, hd + 1, r, pchunk) for r in range(0, S, pchunk)]
            fk = [functools.partial(proj_k, hd + 1, r, pchunk) for r in range(0, S, pchunk)]
            fv = [functools.partial(proj_v, hd + 1, r, 256) for r in range(0, S - rot, 256)]
            attention(hd, False, fq + fk, fv, None, vhead(hd))
            return 0

        def body_c(hd, _):
            fq = [functools.partial(proj_q, hd + 1, r, 256) for r in range(0, S, 256)]
            attention(hd, False, fq, [], None, (), k_pre.at[hd], v_pre.at[hd])
            return 0

        if LA > 1:
            lax.fori_loop(0, LA - 1, body_c, 0)
        if LA >= 3:
            d_wo[1].wait()
            go(*rest)
        lax.fori_loop(LA - 1, G - 1, head_body, 0)
        for d in (d_uk[1], d_uv[1], d_q[1]):
            d.wait()
        extract(wuk_r, 1, wk_s, C)
        extract(wuv_r, 1, wv_s, C)
        extract(wq_r, 1, wq_s, M)
        lax.fori_loop(G - 1, nh - 1, head_body, 0)
        d_mb.wait()
        for d in d_w:
            d.wait()
        mod_v[:, 2 * M:] = _dot(sc8, wmb_v[...])

        G0 = 8
        g_v[pl.ds(0, G0), :] = jnp.zeros((G0, M), F32)
        g_v[pl.ds(S + G0, G0), :] = jnp.zeros((G0, M), F32)

        def b1(r):
            rows = pl.ds(r * RC, RC)
            x1 = x_v[rows, :].astype(F32) + modrow(2) * acc_v[rows, :]
            acc_v[rows, :] = x1
            h2 = _ln(x1) * (1.0 + modrow(4)) + modrow(3)
            h_v[rows, :] = h2.astype(BF16)
            g = _gelu(_dot(_ln(h2).astype(BF16), w1_v[...]))
            g_v[pl.ds(r * RC + G0, RC), :] = g

        outs = []
        c128 = lax.broadcasted_iota(jnp.int32, (RC, 128), 1)

        stB = {}

        def stC(r):
            base = r * RC + G0

            def sh(d, lo):
                return g_v[pl.ds(base + d, RC), lo:lo + 128]
            t0 = sh(-1, 0)
            t1 = jnp.where(c128 < 32, sh(-1, 128), sh(1, 128))
            t2 = jnp.where(c128 < 64, sh(1, 256), sh(-2, 256))
            t3 = jnp.where(c128 < 96, sh(-2, 384), sh(2, 384))
            t4 = sh(2, 512)
            gs = jnp.concatenate([t0, t1, t2, t3, t4], axis=1).astype(BF16)
            rows = pl.ds(r * RC, RC)
            stB[r, 'x1b'] = h_v[rows, :].astype(F32) + _dot(gs, w2_v[...])

        def stD(r):
            stB[r, 'ln'] = _ln(stB[r, 'x1b']).astype(BF16)

        def stE(r):
            stB[r, 'u'] = _gelu(_dot_nt(stB.pop((r, 'ln')), w3_v[...])).astype(BF16)

        def stF(r):
            rows = pl.ds(r * RC, RC)
            y = stB.pop((r, 'x1b')) + _dot(stB.pop((r, 'u')), w4_v[...])
            o_v[rows, :] = (acc_v[rows, :] + modrow(5) * y).astype(BF16)
            oc = pltpu.make_async_copy(o_v.at[rows, :], o_hbm.at[rows, :], sems.at[SEM_O + r])
            oc.start()
            outs.append(oc)

        def stA(r):
            rows = pl.ds(r * RC, RC)
            x1 = x_v[rows, :].astype(F32) + modrow(2) * acc_v[rows, :]
            acc_v[rows, :] = x1
            h2 = _ln(x1) * (1.0 + modrow(4)) + modrow(3)
            h_v[rows, :] = h2.astype(BF16)
            stB[r, 'lnh'] = _ln(h2).astype(BF16)

        def stB1(r):
            g = _gelu(_dot(stB.pop((r, 'lnh')), w1_v[...]))
            g_v[pl.ds(r * RC + G0, RC), :] = g

        NR = S // RC
        if peel:
            attention(H - 1, False, [], [], None, vhead(H - 1))
        if skipB:
            o_v[...] = acc_v[...].astype(BF16)
            oc = pltpu.make_async_copy(o_v, o_hbm, sems.at[SEM_O]); oc.start(); oc.wait()
            return
        seq = []
        if bord == 0:
            seq = [('A', 0), ('B', 0)]
            for r in range(NR):
                seq += [('A', r + 1), ('B', r + 1), ('C', r), ('D', r), ('E', r), ('F', r)]
        elif bord == 1:
            seq = [('A', 0), ('B', 0)]
            for r in range(NR + 1):
                seq += [('A', r + 1), ('B', r + 1), ('C', r), ('D', r), ('F', r - 1), ('E', r)]
        elif bord == 2:
            seq = [('A', 0), ('B', 0), ('A', 1)]
            for r in range(NR + 1):
                seq += [('B', r + 1), ('C', r), ('D', r), ('F', r - 1), ('A', r + 2), ('E', r)]
        elif bord == 3:
            seq = [('A', 0), ('B', 0), ('A', 1)]
            for r in range(NR + 1):
                seq += [('B', r + 1), ('A', r + 2), ('C', r), ('D', r), ('F', r - 1), ('E', r)]
        fnmap = dict(A=stA, B=stB1, C=stC, D=stD, E=stE, F=stF)
        for k, r in seq:
            if 0 <= r < NR:
                fnmap[k](r)
        for oc in outs:
            oc.wait()

    def fn(A_x, A_c_kv, A_w_q, A_w_uk, A_w_uv, A_w_o, B_x, B_w1, B_w2, B_w3, B_w4, c, w_mod):
        x = A_x.reshape(S, M)
        ckv = A_c_kv.reshape(S, C)
        hbm = pl.BlockSpec(memory_space=pltpu.HBM)
        out = pl.pallas_call(
            kernel,
            out_shape=jax.ShapeDtypeStruct((S, M), BF16),
            in_specs=[hbm] * 12 + [pl.BlockSpec(memory_space=pltpu.SMEM)],
            out_specs=hbm,
            scratch_shapes=[
                pltpu.VMEM((S, M), BF16), pltpu.VMEM((S, C), BF16),
                pltpu.VMEM((H // G, M, G // 2, D), U32), pltpu.VMEM((H // G, C, G // 2, D), U32),
                pltpu.VMEM((H // G, C, G // 2, D), U32),
                pltpu.VMEM((H, D, M), BF16),
                pltpu.VMEM((M, M), BF16), pltpu.VMEM((M, M), BF16), pltpu.VMEM((F, M), BF16), pltpu.VMEM((F, M), BF16),
                pltpu.VMEM((1, M), BF16), pltpu.VMEM((M, 2 * M), BF16), pltpu.VMEM((M, 4 * M), BF16),
                pltpu.VMEM((H, M, D), BF16), pltpu.VMEM((H, C, D), BF16), pltpu.VMEM((H, C, D), BF16),
                pltpu.VMEM((8, 6 * M), F32),
                pltpu.VMEM((S, M), BF16),
                pltpu.VMEM((S, D), BF16), pltpu.VMEM((S, D), BF16), pltpu.VMEM((S, D), BF16),
                pltpu.VMEM((max(LA - 1, 1), S, D), BF16), pltpu.VMEM((max(LA - 1, 1), S, D), BF16),
                pltpu.VMEM((S, M), F32),
                pltpu.VMEM((S + 16, M), F32),
                pltpu.VMEM((S, M), BF16),
                pltpu.SemaphoreType.DMA((17 + S // RC,)),
            ],
            compiler_params=pltpu.CompilerParams(vmem_limit_bytes=110 * 1024 * 1024),
        )(x, ckv, A_w_q, A_w_uk, A_w_uv, A_w_o, B_w1, B_w2, B_w3.T, B_w4, c, w_mod, np.zeros((1,), np.int32))
        return out.reshape(1, S, M)
    return jax.jit(fn)


pallas_adaLN_cond__compressed_kv_cla__mixer_s_mlp__prompt_kernel = make()
```

```python
import functools
import jax
import numpy as np
import jax.numpy as jnp
from jax import lax
import jax.experimental.pallas as pl
import jax.experimental.pallas.tpu as pltpu

F32 = jnp.float32
BF16 = jnp.bfloat16
U32 = jnp.uint32
LOG2E = 1.4426950408889634
NEG = -1e9 * LOG2E


def _dot(a, b):
    return jnp.dot(a, b, preferred_element_type=F32)


def _dot_nt(a, b):
    return lax.dot_general(a, b, (((1,), (1,)), ((), ())), preferred_element_type=F32)


def _ln(x):
    m = jnp.mean(x, axis=-1, keepdims=True)
    xc = x - m
    v = jnp.mean(xc * xc, axis=-1, keepdims=True)
    return xc * lax.rsqrt(v + 1e-5)


def _gelu(x):
    return jax.nn.gelu(x, approximate=True)


def make(nh=32, lag=2, pchunk=512, pstart=7, RC=256, border=0, peel=True, finpos=0, skipB=False, stop=0, rot=1536, rotpos=1, pvfirst=1, depm=0, slack=0, finlag=0, bord=2, LA=3, lnpos=0, pro=3, lnc=256, kw=8, vw=6, qw=20, p1=6, p2=14, p3=26):
    S, M, C, H, D, F = 2048, 640, 512, 32, 128, 1728
    BQ = 256
    NQ = S // BQ
    G = 8

    def kernel(x_hbm, ckv_hbm, wq_hbm, wuk_hbm, wuv_hbm, wo_hbm, w1_hbm, w2_hbm, w3_hbm, w4_hbm, c_hbm, wmod_hbm, never_ref,
               o_hbm,
               x_v, ckv_v, wq_r, wuk_r, wuv_r, wo_v, w1_v, w2_v, w3_v, w4_v, c_v, wma_v, wmb_v,
               wq_s, wk_s, wv_s, mod_v, h_v, q_v, k_v, v_v, k_pre, v_pre, acc_v, g_v, o_v, sems):
        NG = H // G
        NW = max(LA - 1, 1)
        PG = G // 2

        def cp(i, src, dst):
            return pltpu.make_async_copy(src, dst, sems.at[i])

        class Multi:
            def __init__(self, ds):
                self.ds = ds

            def start(self):
                for d in self.ds:
                    d.start()

            def wait(self):
                for d in self.ds:
                    d.wait()

        def wcp(i, hbm, raw, g):
            hu = hbm.bitcast(U32)
            return Multi([cp(i + 2 * g + e, hu.at[:, e, pl.ds(PG * g, PG), :], raw.at[g, :, pl.ds(PG * e, PG), :])
                          for e in range(2)])

        d_ckv = cp(0, ckv_hbm, ckv_v)
        d_uk = lambda g: wcp(32, wuk_hbm, wuk_r, g)
        d_uv = lambda g: wcp(40, wuv_hbm, wuv_r, g)
        d_q = lambda g: wcp(48, wq_hbm, wq_r, g)
        d_c = cp(7, c_hbm, c_v)
        d_ma = cp(8, wmod_hbm.at[:, pl.ds(0, 2 * M)], wma_v)
        d_mb = cp(9, wmod_hbm.at[:, pl.ds(2 * M, 4 * M)], wmb_v)
        d_x = cp(10, x_hbm, x_v)
        d_wo = [cp(11, wo_hbm.at[pl.ds(0, NW)], wo_v.at[pl.ds(0, NW)]),
                cp(12, wo_hbm.at[pl.ds(NW, H - NW)], wo_v.at[pl.ds(NW, H - NW)])]
        d_w = [cp(13, w1_hbm, w1_v), cp(14, w2_hbm, w2_v), cp(15, w3_hbm, w3_v), cp(16, w4_hbm, w4_v)]
        SEM_O = 17

        def extract_pair(raw, g, dst, n, j):
            r2 = raw.at[g].reshape(n * PG, D)
            b = r2[pl.ds(j, n, stride=PG), :]
            dst[G * g + 2 * j] = pltpu.bitcast(b << U32(16), F32).astype(BF16)
            dst[G * g + 2 * j + 1] = pltpu.bitcast(b & U32(0xFFFF0000), F32).astype(BF16)

        def extract(raw, g, dst, n):
            for j in range(PG):
                extract_pair(raw, g, dst, n, j)

        qscale = (D ** -0.5) * LOG2E

        def proj_q(hd, r, n):
            rows = pl.ds(r, n)
            q_v[rows, :] = (_dot(h_v[rows, :], wq_s[hd]) * qscale).astype(BF16)

        def proj_k(hd, r, n, dst=None):
            rows = pl.ds(r, n)
            dst = k_v if dst is None else dst
            dst[rows, :] = _dot(ckv_v[rows, :], wk_s[hd]).astype(BF16)

        def proj_v(hd, r, n, dst=None):
            rows = pl.ds(r, n)
            dst = v_v if dst is None else dst
            dst[rows, :] = _dot(ckv_v[rows, :], wv_s[hd]).astype(BF16)

        def modrow(i):
            return mod_v[0:1, i * M:(i + 1) * M]

        def go(*ds):
            for d in ds:
                d.start()

        def ln_a(r):
            rows = pl.ds(r * 256, 256)
            xx = x_v[rows, :].astype(F32)
            h_v[rows, :] = (_ln(xx) * (1.0 + modrow(1)) + modrow(0)).astype(BF16)
            acc_v[rows, :] = jnp.zeros((256, M), F32)

        def kdst(hd):
            return k_v if hd == LA - 1 else k_pre.at[hd]

        def vdst(hd):
            return v_v if hd == LA - 1 else v_pre.at[hd]

        def do_mod():
            cc = c_v[...].astype(F32)
            sc8 = jnp.broadcast_to((cc * jax.nn.sigmoid(cc)).astype(BF16), (8, M))
            mod_v[:, 0:2 * M] = _dot(sc8, wma_v[...])
            return sc8

        def ln_rows(r, n):
            rows = pl.ds(r, n)
            xx = x_v[rows, :].astype(F32)
            h_v[rows, :] = (_ln(xx) * (1.0 + modrow(1)) + modrow(0)).astype(BF16)
            acc_v[rows, :] = jnp.zeros((n, M), F32)

        def interleave(a, b):
            na, nb = len(a), len(b)
            ia = ib = 0
            while ia < na or ib < nb:
                if ib >= nb or (ia < na and ia * max(nb, 1) <= ib * max(na, 1)):
                    a[ia](); ia += 1
                else:
                    b[ib](); ib += 1

        P = functools.partial
        rest = (*[f(g) for g in range(1, NG) for f in (d_uk, d_uv, d_q)], d_mb, *d_w)
        kjobs = [P(proj_k, hd, r, 256, kdst(hd)) for hd in range(LA) for r in range(0, S, 256)]
        vjobs = [P(proj_v, hd, r, 256, vdst(hd)) for hd in range(LA)
                 for r in range(0, S if hd < LA - 1 else S - rot, 256)]
        qjobs = [P(proj_q, 0, r, 256) for r in range(0, S, 256)]
        exk = [P(extract_pair, wuk_r, 0, wk_s, C, j) for j in range(PG)]
        exv = [P(extract_pair, wuv_r, 0, wv_s, C, j) for j in range(PG)]
        exq = [P(extract_pair, wq_r, 0, wq_s, M, j) for j in range(PG)]
        lnj = [P(ln_rows, r, lnc) for r in range(0, S, lnc)]

        def run(js):
            for f in js:
                f()

        def zip_first(ex, jobs):
            out = []
            exi = 0
            for n, f in enumerate(jobs):
                need = (n // 8) // 2 + 1
                want = max(need, min(PG, n + 1))
                while exi < want:
                    out.append(ex[exi]); exi += 1
                out.append(f)
            out += ex[exi:]
            return out

        if pro == 0:
            go(d_ckv, d_uk(0), d_uv(0))
            d_ckv.wait(); d_uk(0).wait()
            go(d_c, d_ma, d_x, d_q(0), d_wo[0])
            run(zip_first(exk, kjobs))
            d_uv(0).wait()
            vz = zip_first(exv, vjobs)
            nv0 = 12
            run(vz[:nv0])
            d_c.wait(); d_ma.wait(); d_x.wait()
            sc8 = do_mod()
            interleave(vz[nv0:], lnj)
            d_q(0).wait()
            go(d_wo[1])
            run(zip_first(exq, qjobs))
        elif pro == 1:
            go(d_ckv, d_uk(0))
            d_ckv.wait(); d_uk(0).wait()
            go(d_uv(0), d_c, d_ma, d_x, d_q(0), d_wo[0])
            run(zip_first(exk, kjobs))
            d_uv(0).wait()
            vz = zip_first(exv, vjobs)
            nv0 = 12
            run(vz[:nv0])
            d_c.wait(); d_ma.wait(); d_x.wait()
            sc8 = do_mod()
            interleave(vz[nv0:], lnj)
            d_q(0).wait()
            go(d_wo[1])
            run(zip_first(exq, qjobs))
        elif pro == 2:
            go(d_c, d_ma, d_x)
            d_c.wait(); d_ma.wait()
            go(d_ckv, d_uk(0))
            sc8 = do_mod()
            d_x.wait()
            go(d_uv(0), d_q(0), d_wo[0])
            run(lnj)
            d_ckv.wait(); d_uk(0).wait()
            run(zip_first(exk, kjobs))
            d_uv(0).wait()
            run(zip_first(exv, vjobs))
            d_q(0).wait()
            go(d_wo[1])
            run(zip_first(exq, qjobs))
        elif pro == 3:
            go(d_ckv, d_uk(0), d_uv(0))
            d_ckv.wait(); d_uk(0).wait()
            go(d_c, d_ma, d_x, d_q(0), d_wo[0])
            nfirst = (LA + 1) // 2
            run(exk[:nfirst])
            interleave(kjobs[:kw], exk[nfirst:])
            d_uv(0).wait()
            interleave(kjobs[kw:], exv)
            run(vjobs[:vw])
            d_c.wait(); d_ma.wait(); d_x.wait()
            sc8 = do_mod()
            interleave(vjobs[vw:qw], lnj)
            d_q(0).wait()
            go(d_wo[1])
            interleave(vjobs[qw:], exq)
            run(qjobs)
        elif pro == 4:
            go(d_ckv, d_uk(0))
            d_ckv.wait(); d_uk(0).wait()
            go(d_uv(0))
            nfirst = (LA + 1) // 2
            run(exk[:nfirst])
            kz = []
            interleave([P(kz.append, f) for f in kjobs[:kw]], [P(kz.append, f) for f in exk[nfirst:]])
            kz += kjobs[kw:]
            marks = {p1: (d_c, d_ma), p2: (d_x,), p3: (d_q(0), d_wo[0])}
            done = set()
            for n, f in enumerate(kz):
                if n in marks:
                    go(*marks[n]); done.add(n)
                f()
            for n in marks:
                if n not in done:
                    go(*marks[n])
            d_uv(0).wait()
            vz = zip_first(exv, vjobs)
            run(vz[:vw])
            d_c.wait(); d_ma.wait(); d_x.wait()
            sc8 = do_mod()
            interleave(vz[vw:], lnj)
            d_q(0).wait()
            go(d_wo[1])
            run(zip_first(exq, qjobs))
        d_wo[0].wait()
        if LA < 3 or stop:
            d_wo[1].wait()
            if stop != 2:
                go(*rest)

        if stop == 1:
            o_v[...] = h_v[...]
            oc = pltpu.make_async_copy(o_v, o_hbm, sems.at[SEM_O]); oc.start(); oc.wait()
            for d in rest:
                d.wait()
            return
        if stop == 2:
            o_v[...] = h_v[...]
            oc = pltpu.make_async_copy(o_v, o_hbm, sems.at[SEM_O]); oc.start(); oc.wait()
            return
        nv = lax.broadcasted_iota(jnp.int32, (BQ, 128), 1) < never_ref[0]
        tri = (lax.broadcasted_iota(jnp.int32, (128, 128), 1) <= lax.broadcasted_iota(jnp.int32, (128, 128), 0))

        def attention(hd, first, fillers_qk, fillers_v, tail, fillers_head=(), k_v=k_v, v_v=v_v):
            wo_h = wo_v[hd]
            st = {}
            hist = []

            def qk(qi, t):
                d = st.setdefault(qi, dict(ss={}, mp=None, lp=None, acc=None))
                q = q_v[pl.ds(qi * BQ, BQ), :]
                if t < qi:
                    s = _dot_nt(q, k_v[pl.ds(t * 256, 256), :])
                    d['ss'][t] = s
                    x = jnp.maximum(s[:, :128], s[:, 128:])
                else:
                    s0 = _dot_nt(q, k_v[pl.ds(t * 256, 128), :])
                    s1 = _dot_nt(q[128:], k_v[pl.ds(t * 256 + 128, 128), :])
                    s0 = jnp.concatenate([jnp.where(tri, s0[:128], NEG), s0[128:]], axis=0)
                    s1 = jnp.where(tri, s1, NEG)
                    d['ss'][t] = (s0, s1)
                    x = jnp.concatenate([s0[:128], jnp.maximum(s0[128:], s1)], axis=0)
                d['mp'] = x if d['mp'] is None else jnp.maximum(d['mp'], x)

            def fin_max(qi):
                m = jnp.max(st[qi]['mp'], axis=-1, keepdims=True)
                st[qi]['m'] = jnp.broadcast_to(m, (BQ, 128))

            def pv(qi, t):
                d = st[qi]
                mm = d['m']
                if len(hist) >= lag and lag > 0:
                    mm = jnp.where(nv, hist[-lag], mm)
                if depm and len(hist) >= 1:
                    mm = jnp.concatenate([mm[:128], jnp.where(nv[:128], hist[-1][:128], mm[128:])], axis=0)
                if t < qi:
                    s = d['ss'][t]
                    p = jnp.exp2(s - jnp.concatenate([mm, mm], axis=1))
                    o = _dot(p.astype(BF16), v_v[pl.ds(t * 256, 256), :])
                    x = p[:, :128] + p[:, 128:]
                else:
                    s0, s1 = d['ss'][t]
                    p0 = jnp.exp2(s0 - mm)
                    p1 = jnp.exp2(s1 - mm[128:])
                    o0 = _dot(p0.astype(BF16), v_v[pl.ds(t * 256, 128), :])
                    o1 = _dot(p1.astype(BF16), v_v[pl.ds(t * 256 + 128, 128), :])
                    o = jnp.concatenate([o0[:128], o0[128:] + o1], axis=0)
                    x = jnp.concatenate([p0[:128], p0[128:] + p1], axis=0)
                hist.append(o)
                d['lp'] = x if d['lp'] is None else d['lp'] + x
                d['acc'] = o if d['acc'] is None else d['acc'] + o

            def fin(qi):
                d = st.pop(qi)
                l = jnp.sum(d['lp'], axis=-1, keepdims=True)
                ctx = (d['acc'] / l).astype(BF16)
                contrib = _dot(ctx, wo_h)
                rows = pl.ds(qi * BQ, BQ)
                if first is True:
                    acc_v[rows, :] = contrib
                elif first is False:
                    acc_v[rows, :] += contrib
                else:
                    acc_v[rows, :] = contrib + jnp.where(first, 0.0, acc_v[rows, :])

            fq = list(fillers_qk)
            fh = list(fillers_head)
            tiles = [(i, t) for i in range(NQ) for t in range(i + 1)]
            qptr = [0]

            def emit_qk_upto(n):
                any_ = False
                while qptr[0] < min(n, len(tiles)):
                    i, t = tiles[qptr[0]]
                    qk(i, t)
                    if fh:
                        fh.pop(0)()
                    if t == i:
                        fin_max(i)
                    qptr[0] += 1
                    any_ = True
                return any_

            def T(i):
                return i * (i + 1) // 2
            emit_qk_upto(1)
            pend_fin = []
            for (qi, t) in tiles:
                if slack == 0:
                    need = T(qi + 1) + t + 1
                    if t == qi:
                        need = T(qi + 2)
                else:
                    need = T(qi + 1) + -(-((t + 1 + slack) * (qi + 2)) // (qi + 1))
                if not pvfirst:
                    if not emit_qk_upto(need) and qptr[0] >= len(tiles) and fq:
                        fq.pop(0)()
                pv(qi, t)
                if pvfirst:
                    if not emit_qk_upto(need) and qptr[0] >= len(tiles) and fq:
                        fq.pop(0)()
                for e in pend_fin:
                    e[0] -= 1
                while pend_fin and pend_fin[0][0] <= 0:
                    fin(pend_fin.pop(0)[1])
                if t == qi:
                    if finlag == 0 or qi == NQ - 1:
                        while pend_fin:
                            fin(pend_fin.pop(0)[1])
                        if qi == NQ - 1:
                            for _ in range(finpos):
                                if fq:
                                    fq.pop(0)()
                        fin(qi)
                    else:
                        pend_fin.append([finlag, qi])
            for f in fq:
                f()
            for f in fillers_v:
                f()

        def vhead(hd):
            return [functools.partial(proj_v, hd, r, 256) for r in range(S - rot, S, 256)]

        def head_body(hd, _):
            fq = [functools.partial(proj_q, hd + 1, r, pchunk) for r in range(0, S, pchunk)]
            fk = [functools.partial(proj_k, hd + 1, r, pchunk) for r in range(0, S, pchunk)]
            fv = [functools.partial(proj_v, hd + 1, r, 256) for r in range(0, S - rot, 256)]
            attention(hd, False, fq + fk, fv, None, vhead(hd))
            return 0

        def body_c(hd, _):
            fq = [functools.partial(proj_q, hd + 1, r, 256) for r in range(0, S, 256)]
            attention(hd, False, fq, [], None, (), k_pre.at[hd], v_pre.at[hd])
            return 0

        if LA > 1:
            lax.fori_loop(0, LA - 1, body_c, 0)
        if LA >= 3:
            d_wo[1].wait()
            go(*rest)
        def group_body(g, _):
            @pl.when(g > 0)
            def _():
                d_uk(g).wait(); d_uv(g).wait(); d_q(g).wait()
                extract(wuk_r, g, wk_s, C)
                extract(wuv_r, g, wv_s, C)
                extract(wq_r, g, wq_s, M)
            lo = jnp.maximum(G * g - 1, LA - 1)
            hi = jnp.minimum(G * g + G - 1, nh - 1)
            lax.fori_loop(lo, hi, head_body, 0)
            return 0
        lax.fori_loop(0, NG, group_body, 0)
        d_mb.wait()
        for d in d_w:
            d.wait()
        mod_v[:, 2 * M:] = _dot(sc8, wmb_v[...])

        G0 = 8
        g_v[pl.ds(0, G0), :] = jnp.zeros((G0, M), F32)
        g_v[pl.ds(S + G0, G0), :] = jnp.zeros((G0, M), F32)

        def b1(r):
            rows = pl.ds(r * RC, RC)
            x1 = x_v[rows, :].astype(F32) + modrow(2) * acc_v[rows, :]
            acc_v[rows, :] = x1
            h2 = _ln(x1) * (1.0 + modrow(4)) + modrow(3)
            h_v[rows, :] = h2.astype(BF16)
            g = _gelu(_dot(_ln(h2).astype(BF16), w1_v[...]))
            g_v[pl.ds(r * RC + G0, RC), :] = g

        outs = []
        c128 = lax.broadcasted_iota(jnp.int32, (RC, 128), 1)

        stB = {}

        def stC(r):
            base = r * RC + G0

            def sh(d, lo):
                return g_v[pl.ds(base + d, RC), lo:lo + 128]
            t0 = sh(-1, 0)
            t1 = jnp.where(c128 < 32, sh(-1, 128), sh(1, 128))
            t2 = jnp.where(c128 < 64, sh(1, 256), sh(-2, 256))
            t3 = jnp.where(c128 < 96, sh(-2, 384), sh(2, 384))
            t4 = sh(2, 512)
            gs = jnp.concatenate([t0, t1, t2, t3, t4], axis=1).astype(BF16)
            rows = pl.ds(r * RC, RC)
            stB[r, 'x1b'] = h_v[rows, :].astype(F32) + _dot(gs, w2_v[...])

        def stD(r):
            stB[r, 'ln'] = _ln(stB[r, 'x1b']).astype(BF16)

        def stE(r):
            stB[r, 'u'] = _gelu(_dot_nt(stB.pop((r, 'ln')), w3_v[...])).astype(BF16)

        def stF(r):
            rows = pl.ds(r * RC, RC)
            y = stB.pop((r, 'x1b')) + _dot(stB.pop((r, 'u')), w4_v[...])
            o_v[rows, :] = (acc_v[rows, :] + modrow(5) * y).astype(BF16)
            oc = pltpu.make_async_copy(o_v.at[rows, :], o_hbm.at[rows, :], sems.at[SEM_O + r])
            oc.start()
            outs.append(oc)

        def stA(r):
            rows = pl.ds(r * RC, RC)
            x1 = x_v[rows, :].astype(F32) + modrow(2) * acc_v[rows, :]
            acc_v[rows, :] = x1
            h2 = _ln(x1) * (1.0 + modrow(4)) + modrow(3)
            h_v[rows, :] = h2.astype(BF16)
            stB[r, 'lnh'] = _ln(h2).astype(BF16)

        def stB1(r):
            g = _gelu(_dot(stB.pop((r, 'lnh')), w1_v[...]))
            g_v[pl.ds(r * RC + G0, RC), :] = g

        NR = S // RC
        if peel:
            attention(H - 1, False, [], [], None, vhead(H - 1))
        if skipB:
            o_v[...] = acc_v[...].astype(BF16)
            oc = pltpu.make_async_copy(o_v, o_hbm, sems.at[SEM_O]); oc.start(); oc.wait()
            return
        seq = []
        if bord == 0:
            seq = [('A', 0), ('B', 0)]
            for r in range(NR):
                seq += [('A', r + 1), ('B', r + 1), ('C', r), ('D', r), ('E', r), ('F', r)]
        elif bord == 1:
            seq = [('A', 0), ('B', 0)]
            for r in range(NR + 1):
                seq += [('A', r + 1), ('B', r + 1), ('C', r), ('D', r), ('F', r - 1), ('E', r)]
        elif bord == 2:
            seq = [('A', 0), ('B', 0), ('A', 1)]
            for r in range(NR + 1):
                seq += [('B', r + 1), ('C', r), ('D', r), ('F', r - 1), ('A', r + 2), ('E', r)]
        elif bord == 3:
            seq = [('A', 0), ('B', 0), ('A', 1)]
            for r in range(NR + 1):
                seq += [('B', r + 1), ('A', r + 2), ('C', r), ('D', r), ('F', r - 1), ('E', r)]
        fnmap = dict(A=stA, B=stB1, C=stC, D=stD, E=stE, F=stF)
        for k, r in seq:
            if 0 <= r < NR:
                fnmap[k](r)
        for oc in outs:
            oc.wait()

    def fn(A_x, A_c_kv, A_w_q, A_w_uk, A_w_uv, A_w_o, B_x, B_w1, B_w2, B_w3, B_w4, c, w_mod):
        x = A_x.reshape(S, M)
        ckv = A_c_kv.reshape(S, C)
        hbm = pl.BlockSpec(memory_space=pltpu.HBM)
        out = pl.pallas_call(
            kernel,
            out_shape=jax.ShapeDtypeStruct((S, M), BF16),
            in_specs=[hbm] * 12 + [pl.BlockSpec(memory_space=pltpu.SMEM)],
            out_specs=hbm,
            scratch_shapes=[
                pltpu.VMEM((S, M), BF16), pltpu.VMEM((S, C), BF16),
                pltpu.VMEM((H // G, M // 2, 8, D), U32), pltpu.VMEM((H // G, C // 2, 8, D), U32),
                pltpu.VMEM((H // G, C // 2, 8, D), U32),
                pltpu.VMEM((H, D, M), BF16),
                pltpu.VMEM((M, M), BF16), pltpu.VMEM((M, M), BF16), pltpu.VMEM((F, M), BF16), pltpu.VMEM((F, M), BF16),
                pltpu.VMEM((1, M), BF16), pltpu.VMEM((M, 2 * M), BF16), pltpu.VMEM((M, 4 * M), BF16),
                pltpu.VMEM((H, M, D), BF16), pltpu.VMEM((H, C, D), BF16), pltpu.VMEM((H, C, D), BF16),
                pltpu.VMEM((8, 6 * M), F32),
                pltpu.VMEM((S, M), BF16),
                pltpu.VMEM((S, D), BF16), pltpu.VMEM((S, D), BF16), pltpu.VMEM((S, D), BF16),
                pltpu.VMEM((max(LA - 1, 1), S, D), BF16), pltpu.VMEM((max(LA - 1, 1), S, D), BF16),
                pltpu.VMEM((S, M), F32),
                pltpu.VMEM((S + 16, M), F32),
                pltpu.VMEM((S, M), BF16),
                pltpu.SemaphoreType.DMA((56,)),
            ],
            compiler_params=pltpu.CompilerParams(vmem_limit_bytes=110 * 1024 * 1024),
        )(x, ckv, A_w_q.reshape(M // 2, 2, H, D), A_w_uk.reshape(C // 2, 2, H, D), A_w_uv.reshape(C // 2, 2, H, D), A_w_o, B_w1, B_w2, B_w3.T, B_w4, c, w_mod, np.zeros((1,), np.int32))
        return out.reshape(1, S, M)
    return jax.jit(fn)


pallas_adaLN_cond__compressed_kv_cla__mixer_s_mlp__prompt_kernel = make(pro=1, LA=3, lnc=128)
```

```python
import functools
import jax
import numpy as np
import jax.numpy as jnp
from jax import lax
import jax.experimental.pallas as pl
import jax.experimental.pallas.tpu as pltpu

F32 = jnp.float32
BF16 = jnp.bfloat16
U32 = jnp.uint32
LOG2E = 1.4426950408889634
NEG = -1e9 * LOG2E


def _dot(a, b):
    return jnp.dot(a, b, preferred_element_type=F32)


def _dot_nt(a, b):
    return lax.dot_general(a, b, (((1,), (1,)), ((), ())), preferred_element_type=F32)


def _ln(x):
    m = jnp.mean(x, axis=-1, keepdims=True)
    xc = x - m
    v = jnp.mean(xc * xc, axis=-1, keepdims=True)
    return xc * lax.rsqrt(v + 1e-5)


def _gelu(x):
    return jax.nn.gelu(x, approximate=True)


def make(nh=32, lag=2, pchunk=512, pstart=7, RC=256, border=0, peel=True, finpos=0, skipB=False, stop=0, rot=1536, rotpos=1, pvfirst=1, depm=0, slack=0, finlag=0, bord=2, LA=4, lnpos=0, pro=5, lnc=64, kw=4, vw=6, qw=20, p1=6, p2=14, p3=26, ford=0, vch=512, bfill=1, qrot=512, qch=256, zinit=0):
    S, M, C, H, D, F = 2048, 640, 512, 32, 128, 1728
    BQ = 256
    NQ = S // BQ
    G = 8

    def kernel(x_hbm, ckv_hbm, wq_hbm, wuk_hbm, wuv_hbm, wo_hbm, w1_hbm, w2_hbm, w3_hbm, w4_hbm, c_hbm, wmod_hbm, never_ref,
               o_hbm,
               x_v, ckv_v, wq_r, wuk_r, wuv_r, wo_v, w1_v, w2_v, w3_v, w4_v, c_v, wma_v, wmb_v,
               wq_s, wk_s, wv_s, mod_v, h_v, q_v, k_v, v_v, k_pre, v_pre, acc_v, g_v, o_v, sems):
        NG = H // G
        NW = max(LA - 1, 1)
        PG = G // 2

        def cp(i, src, dst):
            return pltpu.make_async_copy(src, dst, sems.at[i])

        class Multi:
            def __init__(self, ds):
                self.ds = ds

            def start(self):
                for d in self.ds:
                    d.start()

            def wait(self):
                for d in self.ds:
                    d.wait()

        def wcp(i, hbm, raw, g):
            hu = hbm.bitcast(U32)
            return Multi([cp(i + 2 * g + e, hu.at[:, e, pl.ds(PG * g, PG), :], raw.at[g, :, pl.ds(PG * e, PG), :])
                          for e in range(2)])

        d_ckv = cp(0, ckv_hbm, ckv_v)
        d_uk = lambda g: wcp(32, wuk_hbm, wuk_r, g)
        d_uv = lambda g: wcp(40, wuv_hbm, wuv_r, g)
        d_q = lambda g: wcp(48, wq_hbm, wq_r, g)
        d_c = cp(7, c_hbm, c_v)
        d_ma = cp(8, wmod_hbm.at[:, pl.ds(0, 2 * M)], wma_v)
        d_mb = cp(9, wmod_hbm.at[:, pl.ds(2 * M, 4 * M)], wmb_v)
        d_x = cp(10, x_hbm, x_v)
        d_wo = [cp(11, wo_hbm.at[pl.ds(0, NW)], wo_v.at[pl.ds(0, NW)]),
                cp(12, wo_hbm.at[pl.ds(NW, H - NW)], wo_v.at[pl.ds(NW, H - NW)])]
        d_w = [cp(13, w1_hbm, w1_v), cp(14, w2_hbm, w2_v), cp(15, w3_hbm, w3_v), cp(16, w4_hbm, w4_v)]
        SEM_O = 17

        def extract_pair(raw, g, dst, n, j):
            r2 = raw.at[g].reshape(n * PG, D)
            b = r2[pl.ds(j, n, stride=PG), :]
            dst[G * g + 2 * j] = pltpu.bitcast(b << U32(16), F32).astype(BF16)
            dst[G * g + 2 * j + 1] = pltpu.bitcast(b & U32(0xFFFF0000), F32).astype(BF16)

        def extract(raw, g, dst, n):
            for j in range(PG):
                extract_pair(raw, g, dst, n, j)

        qscale = (D ** -0.5) * LOG2E

        def proj_q(hd, r, n):
            rows = pl.ds(r, n)
            q_v[rows, :] = (_dot(h_v[rows, :], wq_s[hd]) * qscale).astype(BF16)

        def proj_k(hd, r, n, dst=None):
            rows = pl.ds(r, n)
            dst = k_v if dst is None else dst
            dst[rows, :] = _dot(ckv_v[rows, :], wk_s[hd]).astype(BF16)

        def proj_v(hd, r, n, dst=None):
            rows = pl.ds(r, n)
            dst = v_v if dst is None else dst
            dst[rows, :] = _dot(ckv_v[rows, :], wv_s[hd]).astype(BF16)

        def modrow(i):
            return mod_v[0:1, i * M:(i + 1) * M]

        def go(*ds):
            for d in ds:
                d.start()

        def ln_a(r):
            rows = pl.ds(r * 256, 256)
            xx = x_v[rows, :].astype(F32)
            h_v[rows, :] = (_ln(xx) * (1.0 + modrow(1)) + modrow(0)).astype(BF16)
            acc_v[rows, :] = jnp.zeros((256, M), F32)

        def kdst(hd):
            return k_v if hd == LA - 1 else k_pre.at[hd]

        def vdst(hd):
            return v_v if hd == LA - 1 else v_pre.at[hd]

        def do_mod():
            cc = c_v[...].astype(F32)
            sc8 = jnp.broadcast_to((cc * jax.nn.sigmoid(cc)).astype(BF16), (8, M))
            mod_v[:, 0:2 * M] = _dot(sc8, wma_v[...])
            return sc8

        def ln_rows(r, n):
            rows = pl.ds(r, n)
            xx = x_v[rows, :].astype(F32)
            h_v[rows, :] = (_ln(xx) * (1.0 + modrow(1)) + modrow(0)).astype(BF16)
            if zinit:
                acc_v[rows, :] = jnp.zeros((n, M), F32)

        def interleave(a, b):
            na, nb = len(a), len(b)
            ia = ib = 0
            while ia < na or ib < nb:
                if ib >= nb or (ia < na and ia * max(nb, 1) <= ib * max(na, 1)):
                    a[ia](); ia += 1
                else:
                    b[ib](); ib += 1

        P = functools.partial
        rest = (*[f(g) for g in range(1, NG) for f in (d_uk, d_uv, d_q)], d_mb, *d_w)
        kjobs = [P(proj_k, hd, r, 256, kdst(hd)) for hd in range(LA) for r in range(0, S, 256)]
        vjobs = [P(proj_v, hd, r, 256, vdst(hd)) for hd in range(LA)
                 for r in range(0, S if hd < LA - 1 else S - rot, 256)]
        qjobs = [P(proj_q, 0, r, 256) for r in range(0, S - qrot, 256)]
        exk = [P(extract_pair, wuk_r, 0, wk_s, C, j) for j in range(PG)]
        exv = [P(extract_pair, wuv_r, 0, wv_s, C, j) for j in range(PG)]
        exq = [P(extract_pair, wq_r, 0, wq_s, M, j) for j in range(PG)]
        lnj = [P(ln_rows, r, lnc) for r in range(0, S, lnc)]

        def run(js):
            for f in js:
                f()

        def zip_first(ex, jobs):
            out = []
            exi = 0
            for n, f in enumerate(jobs):
                need = min((n // 8) // 2 + 1, PG)
                want = max(need, min(PG, n + 1))
                while exi < want:
                    out.append(ex[exi]); exi += 1
                out.append(f)
            out += ex[exi:]
            return out

        if pro == 0:
            go(d_ckv, d_uk(0), d_uv(0))
            d_ckv.wait(); d_uk(0).wait()
            go(d_c, d_ma, d_x, d_q(0), d_wo[0])
            run(zip_first(exk, kjobs))
            d_uv(0).wait()
            vz = zip_first(exv, vjobs)
            nv0 = 12
            run(vz[:nv0])
            d_c.wait(); d_ma.wait(); d_x.wait()
            sc8 = do_mod()
            interleave(vz[nv0:], lnj)
            d_q(0).wait()
            go(d_wo[1])
            run(zip_first(exq, qjobs))
        elif pro == 1:
            go(d_ckv, d_uk(0))
            d_ckv.wait(); d_uk(0).wait()
            go(d_uv(0), d_c, d_ma, d_x, d_q(0), d_wo[0])
            run(zip_first(exk, kjobs))
            d_uv(0).wait()
            vz = zip_first(exv, vjobs)
            nv0 = 12
            run(vz[:nv0])
            d_c.wait(); d_ma.wait(); d_x.wait()
            sc8 = do_mod()
            interleave(vz[nv0:], lnj)
            d_q(0).wait()
            go(d_wo[1])
            run(zip_first(exq, qjobs))
        elif pro == 2:
            go(d_c, d_ma, d_x)
            d_c.wait(); d_ma.wait()
            go(d_ckv, d_uk(0))
            sc8 = do_mod()
            d_x.wait()
            go(d_uv(0), d_q(0), d_wo[0])
            run(lnj)
            d_ckv.wait(); d_uk(0).wait()
            run(zip_first(exk, kjobs))
            d_uv(0).wait()
            run(zip_first(exv, vjobs))
            d_q(0).wait()
            go(d_wo[1])
            run(zip_first(exq, qjobs))
        elif pro == 3:
            go(d_ckv, d_uk(0), d_uv(0))
            d_ckv.wait(); d_uk(0).wait()
            go(d_c, d_ma, d_x, d_q(0), d_wo[0])
            nfirst = (LA + 1) // 2
            run(exk[:nfirst])
            interleave(kjobs[:kw], exk[nfirst:])
            d_uv(0).wait()
            interleave(kjobs[kw:], exv)
            run(vjobs[:vw])
            d_c.wait(); d_ma.wait(); d_x.wait()
            sc8 = do_mod()
            interleave(vjobs[vw:qw], lnj)
            d_q(0).wait()
            go(d_wo[1])
            interleave(vjobs[qw:], exq)
            run(qjobs)
        elif pro == 4:
            go(d_ckv, d_uk(0))
            d_ckv.wait(); d_uk(0).wait()
            go(d_uv(0))
            nfirst = (LA + 1) // 2
            run(exk[:nfirst])
            kz = []
            interleave([P(kz.append, f) for f in kjobs[:kw]], [P(kz.append, f) for f in exk[nfirst:]])
            kz += kjobs[kw:]
            marks = {p1: (d_c, d_ma), p2: (d_x,), p3: (d_q(0), d_wo[0])}
            done = set()
            for n, f in enumerate(kz):
                if n in marks:
                    go(*marks[n]); done.add(n)
                f()
            for n in marks:
                if n not in done:
                    go(*marks[n])
            d_uv(0).wait()
            vz = zip_first(exv, vjobs)
            run(vz[:vw])
            d_c.wait(); d_ma.wait(); d_x.wait()
            sc8 = do_mod()
            interleave(vz[vw:], lnj)
            d_q(0).wait()
            go(d_wo[1])
            run(zip_first(exq, qjobs))
        elif pro == 5:
            go(d_ckv, d_uk(0))
            d_ckv.wait(); d_uk(0).wait()
            go(d_uv(0), d_c, d_ma, d_x)
            kz = zip_first(exk, kjobs)
            for n, f in enumerate(kz):
                if n == p1:
                    go(d_q(0), d_wo[0])
                if n == len(kz) - kw:
                    d_uv(0).wait()
                    kz2 = []
                    interleave([P(kz2.append, f2) for f2 in kz[n:]], [P(kz2.append, f2) for f2 in exv])
                    run(kz2)
                    break
                f()
            run(vjobs[:8])
            d_c.wait(); d_ma.wait(); d_x.wait()
            sc8 = do_mod()
            NI = 2

            def vl(i, _):
                r0 = pl.multiple_of(i * (S // NI), S // NI)
                r1 = pl.multiple_of(i * ((S - rot) // NI), 128)
                nl = (S // NI) // lnc
                jobs = []
                for hd in range(1, LA - 1):
                    for r in range(0, S // NI, 256):
                        jobs.append(P(proj_v, hd, r0 + r, 256, vdst(hd)))
                jobs.append(P(proj_v, LA - 1, r1, (S - rot) // NI, vdst(LA - 1)))
                interleave(jobs, [P(ln_rows, r0 + k * lnc, lnc) for k in range(nl)])
                return 0
            lax.fori_loop(0, NI, vl, 0)
            d_q(0).wait()
            go(d_wo[1])
            run(zip_first(exq, qjobs))
        d_wo[0].wait()
        if LA < 3 or stop:
            d_wo[1].wait()
            if stop != 2:
                go(*rest)

        if stop == 1:
            o_v[...] = h_v[...]
            oc = pltpu.make_async_copy(o_v, o_hbm, sems.at[SEM_O]); oc.start(); oc.wait()
            for d in rest:
                d.wait()
            return
        if stop == 2:
            o_v[...] = h_v[...]
            oc = pltpu.make_async_copy(o_v, o_hbm, sems.at[SEM_O]); oc.start(); oc.wait()
            return
        nv = lax.broadcasted_iota(jnp.int32, (BQ, 128), 1) < never_ref[0]
        tri = (lax.broadcasted_iota(jnp.int32, (128, 128), 1) <= lax.broadcasted_iota(jnp.int32, (128, 128), 0))

        def attention(hd, first, fillers_qk, fillers_v, tail, fillers_head=(), k_v=k_v, v_v=v_v):
            wo_h = wo_v[hd]
            st = {}
            hist = []

            def qk(qi, t):
                d = st.setdefault(qi, dict(ss={}, mp=None, lp=None, acc=None))
                q = q_v[pl.ds(qi * BQ, BQ), :]
                if t < qi:
                    s = _dot_nt(q, k_v[pl.ds(t * 256, 256), :])
                    d['ss'][t] = s
                    x = jnp.maximum(s[:, :128], s[:, 128:])
                else:
                    s0 = _dot_nt(q, k_v[pl.ds(t * 256, 128), :])
                    s1 = _dot_nt(q[128:], k_v[pl.ds(t * 256 + 128, 128), :])
                    s0 = jnp.concatenate([jnp.where(tri, s0[:128], NEG), s0[128:]], axis=0)
                    s1 = jnp.where(tri, s1, NEG)
                    d['ss'][t] = (s0, s1)
                    x = jnp.concatenate([s0[:128], jnp.maximum(s0[128:], s1)], axis=0)
                d['mp'] = x if d['mp'] is None else jnp.maximum(d['mp'], x)

            def fin_max(qi):
                m = jnp.max(st[qi]['mp'], axis=-1, keepdims=True)
                st[qi]['m'] = jnp.broadcast_to(m, (BQ, 128))

            def pv(qi, t):
                d = st[qi]
                mm = d['m']
                if len(hist) >= lag and lag > 0:
                    mm = jnp.where(nv, hist[-lag], mm)
                if depm and len(hist) >= 1:
                    mm = jnp.concatenate([mm[:128], jnp.where(nv[:128], hist[-1][:128], mm[128:])], axis=0)
                if t < qi:
                    s = d['ss'][t]
                    p = jnp.exp2(s - jnp.concatenate([mm, mm], axis=1))
                    o = _dot(p.astype(BF16), v_v[pl.ds(t * 256, 256), :])
                    x = p[:, :128] + p[:, 128:]
                else:
                    s0, s1 = d['ss'][t]
                    p0 = jnp.exp2(s0 - mm)
                    p1 = jnp.exp2(s1 - mm[128:])
                    o0 = _dot(p0.astype(BF16), v_v[pl.ds(t * 256, 128), :])
                    o1 = _dot(p1.astype(BF16), v_v[pl.ds(t * 256 + 128, 128), :])
                    o = jnp.concatenate([o0[:128], o0[128:] + o1], axis=0)
                    x = jnp.concatenate([p0[:128], p0[128:] + p1], axis=0)
                hist.append(o)
                d['lp'] = x if d['lp'] is None else d['lp'] + x
                d['acc'] = o if d['acc'] is None else d['acc'] + o

            def fin(qi):
                d = st.pop(qi)
                l = jnp.sum(d['lp'], axis=-1, keepdims=True)
                ctx = (d['acc'] / l).astype(BF16)
                contrib = _dot(ctx, wo_h)
                rows = pl.ds(qi * BQ, BQ)
                if first is True:
                    acc_v[rows, :] = contrib
                elif first is False:
                    acc_v[rows, :] += contrib
                else:
                    acc_v[rows, :] = contrib + jnp.where(first, 0.0, acc_v[rows, :])

            fq = list(fillers_qk)
            fh = list(fillers_head)
            tiles = [(i, t) for i in range(NQ) for t in range(i + 1)]
            qptr = [0]

            def emit_qk_upto(n):
                any_ = False
                while qptr[0] < min(n, len(tiles)):
                    i, t = tiles[qptr[0]]
                    qk(i, t)
                    if fh:
                        fh.pop(0)()
                    if t == i:
                        fin_max(i)
                    qptr[0] += 1
                    any_ = True
                return any_

            def T(i):
                return i * (i + 1) // 2
            emit_qk_upto(1)
            pend_fin = []
            for (qi, t) in tiles:
                if slack == 0:
                    need = T(qi + 1) + t + 1
                    if t == qi:
                        need = T(qi + 2)
                else:
                    need = T(qi + 1) + -(-((t + 1 + slack) * (qi + 2)) // (qi + 1))
                if not pvfirst:
                    if not emit_qk_upto(need) and qptr[0] >= len(tiles) and fq:
                        fq.pop(0)()
                pv(qi, t)
                if pvfirst:
                    if not emit_qk_upto(need) and qptr[0] >= len(tiles) and fq:
                        fq.pop(0)()
                for e in pend_fin:
                    e[0] -= 1
                while pend_fin and pend_fin[0][0] <= 0:
                    fin(pend_fin.pop(0)[1])
                if t == qi:
                    if finlag == 0 or qi == NQ - 1:
                        while pend_fin:
                            fin(pend_fin.pop(0)[1])
                        if qi == NQ - 1:
                            for _ in range(finpos):
                                if fq:
                                    fq.pop(0)()
                        fin(qi)
                    else:
                        pend_fin.append([finlag, qi])
            for f in fq:
                f()
            for f in fillers_v:
                f()

        def vhead(hd):
            return [functools.partial(proj_v, hd, r, vch) for r in range(S - rot, S, vch)]

        def head_body(hd, _):
            fq = [functools.partial(proj_q, hd + 1, r, pchunk) for r in range(0, S, pchunk)]
            fk = [functools.partial(proj_k, hd + 1, r, pchunk) for r in range(0, S, pchunk)]
            fv = [functools.partial(proj_v, hd + 1, r, vch) for r in range(0, S - rot, vch)]
            if ford == 0:
                ff = fq + fk
            elif ford == 1:
                ff = fk + fq
            else:
                ff = [f for pr in zip(fq, fk) for f in pr]
            attention(hd, False, ff, fv, None, vhead(hd))
            return 0

        def body_c(hd, _):
            fq = [functools.partial(proj_q, hd + 1, r, qch) for r in range(0, S - qrot, qch)]
            fhq = [functools.partial(proj_q, hd, r, qch) for r in range(S - qrot, S, qch)]
            attention(hd, False if zinit else (hd == 0), fq, [], None, fhq, k_pre.at[hd], v_pre.at[hd])
            return 0

        if LA > 1:
            lax.fori_loop(0, LA - 1, body_c, 0)
            for r in range(S - qrot, S, 512):
                proj_q(LA - 1, r, 512)
        if LA >= 3:
            d_wo[1].wait()
            go(*rest)
        def group_body(g, _):
            @pl.when(g > 0)
            def _():
                d_uk(g).wait(); d_uv(g).wait(); d_q(g).wait()
                extract(wuk_r, g, wk_s, C)
                extract(wuv_r, g, wv_s, C)
                extract(wq_r, g, wq_s, M)
            lo = jnp.maximum(G * g - 1, LA - 1)
            hi = jnp.minimum(G * g + G - 1, nh - 1)
            lax.fori_loop(lo, hi, head_body, 0)
            return 0
        lax.fori_loop(0, NG, group_body, 0)
        d_mb.wait()
        for d in d_w:
            d.wait()
        mod_v[:, 2 * M:] = _dot(sc8, wmb_v[...])

        G0 = 8
        g_v[pl.ds(0, G0), :] = jnp.zeros((G0, M), F32)
        g_v[pl.ds(S + G0, G0), :] = jnp.zeros((G0, M), F32)

        def b1(r):
            rows = pl.ds(r * RC, RC)
            x1 = x_v[rows, :].astype(F32) + modrow(2) * acc_v[rows, :]
            acc_v[rows, :] = x1
            h2 = _ln(x1) * (1.0 + modrow(4)) + modrow(3)
            h_v[rows, :] = h2.astype(BF16)
            g = _gelu(_dot(_ln(h2).astype(BF16), w1_v[...]))
            g_v[pl.ds(r * RC + G0, RC), :] = g

        outs = []
        c128 = lax.broadcasted_iota(jnp.int32, (RC, 128), 1)

        stB = {}

        def stC(r):
            base = r * RC + G0

            def sh(d, lo):
                return g_v[pl.ds(base + d, RC), lo:lo + 128]
            t0 = sh(-1, 0)
            t1 = jnp.where(c128 < 32, sh(-1, 128), sh(1, 128))
            t2 = jnp.where(c128 < 64, sh(1, 256), sh(-2, 256))
            t3 = jnp.where(c128 < 96, sh(-2, 384), sh(2, 384))
            t4 = sh(2, 512)
            gs = jnp.concatenate([t0, t1, t2, t3, t4], axis=1).astype(BF16)
            rows = pl.ds(r * RC, RC)
            stB[r, 'x1b'] = h_v[rows, :].astype(F32) + _dot(gs, w2_v[...])

        def stD(r):
            stB[r, 'ln'] = _ln(stB[r, 'x1b']).astype(BF16)

        def stE(r):
            stB[r, 'u'] = _gelu(_dot_nt(stB.pop((r, 'ln')), w3_v[...])).astype(BF16)

        def stF(r):
            rows = pl.ds(r * RC, RC)
            y = stB.pop((r, 'x1b')) + _dot(stB.pop((r, 'u')), w4_v[...])
            o_v[rows, :] = (acc_v[rows, :] + modrow(5) * y).astype(BF16)
            oc = pltpu.make_async_copy(o_v.at[rows, :], o_hbm.at[rows, :], sems.at[SEM_O + r])
            oc.start()
            outs.append(oc)

        def stA(r):
            rows = pl.ds(r * RC, RC)
            x1 = x_v[rows, :].astype(F32) + modrow(2) * acc_v[rows, :]
            acc_v[rows, :] = x1
            h2 = _ln(x1) * (1.0 + modrow(4)) + modrow(3)
            h_v[rows, :] = h2.astype(BF16)
            stB[r, 'lnh'] = _ln(h2).astype(BF16)

        def stB1(r):
            g = _gelu(_dot(stB.pop((r, 'lnh')), w1_v[...]))
            g_v[pl.ds(r * RC + G0, RC), :] = g

        NR = S // RC
        if skipB:
            o_v[...] = acc_v[...].astype(BF16)
            oc = pltpu.make_async_copy(o_v, o_hbm, sems.at[SEM_O]); oc.start(); oc.wait()
            return
        seq = []
        if bord == 0:
            seq = [('A', 0), ('B', 0)]
            for r in range(NR):
                seq += [('A', r + 1), ('B', r + 1), ('C', r), ('D', r), ('E', r), ('F', r)]
        elif bord == 1:
            seq = [('A', 0), ('B', 0)]
            for r in range(NR + 1):
                seq += [('A', r + 1), ('B', r + 1), ('C', r), ('D', r), ('F', r - 1), ('E', r)]
        elif bord == 2:
            seq = [('A', 0), ('B', 0), ('A', 1)]
            for r in range(NR + 1):
                seq += [('B', r + 1), ('C', r), ('D', r), ('F', r - 1), ('A', r + 2), ('E', r)]
        elif bord == 3:
            seq = [('A', 0), ('B', 0), ('A', 1)]
            for r in range(NR + 1):
                seq += [('B', r + 1), ('A', r + 2), ('C', r), ('D', r), ('F', r - 1), ('E', r)]
        fnmap = dict(A=stA, B=stB1, C=stC, D=stD, E=stE, F=stF)
        bjobs = [functools.partial(fnmap[k], r) for k, r in seq if 0 <= r < NR]
        if bfill:
            attention(H - 1, False, bjobs, [], None, vhead(H - 1))
        else:
            attention(H - 1, False, [], [], None, vhead(H - 1))
            for f in bjobs:
                f()
        for oc in outs:
            oc.wait()

    def fn(A_x, A_c_kv, A_w_q, A_w_uk, A_w_uv, A_w_o, B_x, B_w1, B_w2, B_w3, B_w4, c, w_mod):
        x = A_x.reshape(S, M)
        ckv = A_c_kv.reshape(S, C)
        hbm = pl.BlockSpec(memory_space=pltpu.HBM)
        out = pl.pallas_call(
            kernel,
            out_shape=jax.ShapeDtypeStruct((S, M), BF16),
            in_specs=[hbm] * 12 + [pl.BlockSpec(memory_space=pltpu.SMEM)],
            out_specs=hbm,
            scratch_shapes=[
                pltpu.VMEM((S, M), BF16), pltpu.VMEM((S, C), BF16),
                pltpu.VMEM((H // G, M // 2, 8, D), U32), pltpu.VMEM((H // G, C // 2, 8, D), U32),
                pltpu.VMEM((H // G, C // 2, 8, D), U32),
                pltpu.VMEM((H, D, M), BF16),
                pltpu.VMEM((M, M), BF16), pltpu.VMEM((M, M), BF16), pltpu.VMEM((F, M), BF16), pltpu.VMEM((F, M), BF16),
                pltpu.VMEM((1, M), BF16), pltpu.VMEM((M, 2 * M), BF16), pltpu.VMEM((M, 4 * M), BF16),
                pltpu.VMEM((H, M, D), BF16), pltpu.VMEM((H, C, D), BF16), pltpu.VMEM((H, C, D), BF16),
                pltpu.VMEM((8, 6 * M), F32),
                pltpu.VMEM((S, M), BF16),
                pltpu.VMEM((S, D), BF16), pltpu.VMEM((S, D), BF16), pltpu.VMEM((S, D), BF16),
                pltpu.VMEM((max(LA - 1, 1), S, D), BF16), pltpu.VMEM((max(LA - 1, 1), S, D), BF16),
                pltpu.VMEM((S, M), F32),
                pltpu.VMEM((S + 16, M), F32),
                pltpu.VMEM((S, M), BF16),
                pltpu.SemaphoreType.DMA((56,)),
            ],
            compiler_params=pltpu.CompilerParams(vmem_limit_bytes=110 * 1024 * 1024),
        )(x, ckv, A_w_q.reshape(M // 2, 2, H, D), A_w_uk.reshape(C // 2, 2, H, D), A_w_uv.reshape(C // 2, 2, H, D), A_w_o, B_w1, B_w2, B_w3.T, B_w4, c, w_mod, np.zeros((1,), np.int32))
        return out.reshape(1, S, M)
    return jax.jit(fn)


pallas_adaLN_cond__compressed_kv_cla__mixer_s_mlp__prompt_kernel = make()
```

```python
import functools

import jax
import jax.numpy as jnp
import numpy as np
from jax import lax
import jax.experimental.pallas as pl
import jax.experimental.pallas.tpu as pltpu

F32 = jnp.float32
BF16 = jnp.bfloat16
U32 = jnp.uint32
LOG2E = 1.4426950408889634
NEG = -1e9 * LOG2E

S, M, C, H, D, F = 2048, 640, 512, 32, 128, 1728
BQ = 256
NQ = S // BQ
G = 8
NG = H // G
PG = G // 2
LA = 4
LAG = 2
ROT = 1536
QROT = 512
PCH = 512
RC = 256
NR = S // RC
G0 = 8


def _dot(a, b):
    return jnp.dot(a, b, preferred_element_type=F32)


def _dot_nt(a, b):
    return lax.dot_general(a, b, (((1,), (1,)), ((), ())), preferred_element_type=F32)


def _ln(x):
    m = jnp.mean(x, axis=-1, keepdims=True)
    xc = x - m
    v = jnp.mean(xc * xc, axis=-1, keepdims=True)
    return xc * lax.rsqrt(v + 1e-5)


def _gelu(x):
    return jax.nn.gelu(x, approximate=True)


class _Multi:
    def __init__(self, ds):
        self.ds = ds

    def start(self):
        for d in self.ds:
            d.start()

    def wait(self):
        for d in self.ds:
            d.wait()


def _interleave(a, b):
    na, nb = len(a), len(b)
    ia = ib = 0
    out = []
    while ia < na or ib < nb:
        if ib >= nb or (ia < na and ia * max(nb, 1) <= ib * max(na, 1)):
            out.append(a[ia])
            ia += 1
        else:
            out.append(b[ib])
            ib += 1
    return out


def _run(jobs):
    for f in jobs:
        f()


def _kernel(x_hbm, ckv_hbm, wq_hbm, wuk_hbm, wuv_hbm, wo_hbm, w1_hbm, w2_hbm, w3_hbm, w4_hbm, c_hbm, wmod_hbm,
            zero_ref, o_hbm,
            x_v, ckv_v, wq_r, wuk_r, wuv_r, wo_v, w1_v, w2_v, w3_v, w4_v, c_v, wma_v, wmb_v,
            wq_s, wk_s, wv_s, mod_v, h_v, q_v, k_v, v_v, k_pre, v_pre, acc_v, g_v, o_v, sems):
    P = functools.partial

    def cp(i, src, dst):
        return pltpu.make_async_copy(src, dst, sems.at[i])

    def wcp(i, hbm, raw, g):
        hu = hbm.bitcast(U32)
        return _Multi([cp(i + 2 * g + e, hu.at[:, e, pl.ds(PG * g, PG), :], raw.at[g, :, pl.ds(PG * e, PG), :])
                       for e in range(2)])

    NW = LA - 1
    d_ckv = cp(0, ckv_hbm, ckv_v)
    d_uk = lambda g: wcp(32, wuk_hbm, wuk_r, g)
    d_uv = lambda g: wcp(40, wuv_hbm, wuv_r, g)
    d_q = lambda g: wcp(48, wq_hbm, wq_r, g)
    d_c = cp(7, c_hbm, c_v)
    d_ma = cp(8, wmod_hbm.at[:, pl.ds(0, 2 * M)], wma_v)
    d_mb = cp(9, wmod_hbm.at[:, pl.ds(2 * M, 4 * M)], wmb_v)
    d_x = cp(10, x_hbm, x_v)
    d_wo0 = cp(11, wo_hbm.at[pl.ds(0, NW)], wo_v.at[pl.ds(0, NW)])
    d_wo1 = cp(12, wo_hbm.at[pl.ds(NW, H - NW)], wo_v.at[pl.ds(NW, H - NW)])
    d_w = [cp(13, w1_hbm, w1_v), cp(14, w2_hbm, w2_v), cp(15, w3_hbm, w3_v), cp(16, w4_hbm, w4_v)]
    SEM_O = 17

    def go(*ds):
        for d in ds:
            d.start()

    def extract_pair(raw, g, dst, n, j):
        r2 = raw.at[g].reshape(n * PG, D)
        b = r2[pl.ds(j, n, stride=PG), :]
        dst[G * g + 2 * j] = pltpu.bitcast(b << U32(16), F32).astype(BF16)
        dst[G * g + 2 * j + 1] = pltpu.bitcast(b & U32(0xFFFF0000), F32).astype(BF16)

    def extract(raw, g, dst, n):
        for j in range(PG):
            extract_pair(raw, g, dst, n, j)

    qscale = (D ** -0.5) * LOG2E

    def proj_q(hd, r, n):
        rows = pl.ds(r, n)
        q_v[rows, :] = (_dot(h_v[rows, :], wq_s[hd]) * qscale).astype(BF16)

    def proj_k(hd, r, n, dst=None):
        rows = pl.ds(r, n)
        dst = k_v if dst is None else dst
        dst[rows, :] = _dot(ckv_v[rows, :], wk_s[hd]).astype(BF16)

    def proj_v(hd, r, n, dst=None):
        rows = pl.ds(r, n)
        dst = v_v if dst is None else dst
        dst[rows, :] = _dot(ckv_v[rows, :], wv_s[hd]).astype(BF16)

    def modrow(i):
        return mod_v[0:1, i * M:(i + 1) * M]

    def ln_rows(r, n):
        rows = pl.ds(r, n)
        xx = x_v[rows, :].astype(F32)
        h_v[rows, :] = (_ln(xx) * (1.0 + modrow(1)) + modrow(0)).astype(BF16)

    def kdst(hd):
        return k_v if hd == LA - 1 else k_pre.at[hd]

    def vdst(hd):
        return v_v if hd == LA - 1 else v_pre.at[hd]

    def zip_first(ex, jobs):
        out = []
        exi = 0
        for n, f in enumerate(jobs):
            need = min((n // 8) // 2 + 1, PG)
            want = max(need, min(PG, n + 1))
            while exi < want:
                out.append(ex[exi])
                exi += 1
            out.append(f)
        return out + ex[exi:]

    kjobs = [P(proj_k, hd, r, 256, kdst(hd)) for hd in range(LA) for r in range(0, S, 256)]
    qjobs = [P(proj_q, 0, r, 256) for r in range(0, S - QROT, 256)]
    exk = [P(extract_pair, wuk_r, 0, wk_s, C, j) for j in range(PG)]
    exv = [P(extract_pair, wuv_r, 0, wv_s, C, j) for j in range(PG)]
    exq = [P(extract_pair, wq_r, 0, wq_s, M, j) for j in range(PG)]

    go(d_uk(0), d_ckv)
    d_uk(0).wait()
    kz = zip_first(exk, kjobs)
    for n, f in enumerate(kz):
        if n == 1:
            d_ckv.wait()
            go(d_uv(0), d_c, d_ma, d_x)
        if n == 6:
            go(d_q(0), d_wo0)
        if n == len(kz) - 4:
            d_uv(0).wait()
            _run(_interleave(kz[n:], exv))
            break
        f()
    _run([P(proj_v, 0, r, 256, vdst(0)) for r in range(0, S, 256)])
    d_c.wait()
    d_ma.wait()
    d_x.wait()
    cc = c_v[...].astype(F32)
    sc8 = jnp.broadcast_to((cc * jax.nn.sigmoid(cc)).astype(BF16), (8, M))
    mod_v[:, 0:2 * M] = _dot(sc8, wma_v[...])
    NI, LNC = 2, 64

    def v_ln(i, _):
        r0 = pl.multiple_of(i * (S // NI), S // NI)
        r1 = pl.multiple_of(i * ((S - ROT) // NI), 128)
        jobs = [P(proj_v, hd, r0 + r, 256, vdst(hd)) for hd in range(1, LA - 1) for r in range(0, S // NI, 256)]
        jobs.append(P(proj_v, LA - 1, r1, (S - ROT) // NI, vdst(LA - 1)))
        _run(_interleave(jobs, [P(ln_rows, r0 + k * LNC, LNC) for k in range((S // NI) // LNC)]))
        return 0

    lax.fori_loop(0, NI, v_ln, 0)
    d_q(0).wait()
    go(d_wo1)
    _run(zip_first(exq, qjobs))
    d_wo0.wait()

    never = lax.broadcasted_iota(jnp.int32, (BQ, 128), 1) < zero_ref[0]
    tri = lax.broadcasted_iota(jnp.int32, (128, 128), 1) <= lax.broadcasted_iota(jnp.int32, (128, 128), 0)

    def attention(hd, first, fillers_qk, fillers_v, fillers_head, k_ref, v_ref):
        wo_h = wo_v[hd]
        st = {}
        hist = []

        def qk(qi, t):
            d = st.setdefault(qi, dict(ss={}, mp=None, lp=None, acc=None))
            q = q_v[pl.ds(qi * BQ, BQ), :]
            if t < qi:
                s = _dot_nt(q, k_ref[pl.ds(t * 256, 256), :])
                d['ss'][t] = s
                x = jnp.maximum(s[:, :128], s[:, 128:])
            else:
                s0 = _dot_nt(q, k_ref[pl.ds(t * 256, 128), :])
                s1 = _dot_nt(q[128:], k_ref[pl.ds(t * 256 + 128, 128), :])
                s0 = jnp.concatenate([jnp.where(tri, s0[:128], NEG), s0[128:]], axis=0)
                s1 = jnp.where(tri, s1, NEG)
                d['ss'][t] = (s0, s1)
                x = jnp.concatenate([s0[:128], jnp.maximum(s0[128:], s1)], axis=0)
            d['mp'] = x if d['mp'] is None else jnp.maximum(d['mp'], x)

        def fin_max(qi):
            m = jnp.max(st[qi]['mp'], axis=-1, keepdims=True)
            st[qi]['m'] = jnp.broadcast_to(m, (BQ, 128))

        def pv(qi, t):
            d = st[qi]
            mm = d['m']
            if len(hist) >= LAG:
                mm = jnp.where(never, hist[-LAG], mm)
            if t < qi:
                p = jnp.exp2(d['ss'][t] - jnp.concatenate([mm, mm], axis=1))
                o = _dot(p.astype(BF16), v_ref[pl.ds(t * 256, 256), :])
                x = p[:, :128] + p[:, 128:]
            else:
                s0, s1 = d['ss'][t]
                p0 = jnp.exp2(s0 - mm)
                p1 = jnp.exp2(s1 - mm[128:])
                o0 = _dot(p0.astype(BF16), v_ref[pl.ds(t * 256, 128), :])
                o1 = _dot(p1.astype(BF16), v_ref[pl.ds(t * 256 + 128, 128), :])
                o = jnp.concatenate([o0[:128], o0[128:] + o1], axis=0)
                x = jnp.concatenate([p0[:128], p0[128:] + p1], axis=0)
            hist.append(o)
            d['lp'] = x if d['lp'] is None else d['lp'] + x
            d['acc'] = o if d['acc'] is None else d['acc'] + o

        def fin(qi):
            d = st.pop(qi)
            l = jnp.sum(d['lp'], axis=-1, keepdims=True)
            ctx = (d['acc'] / l).astype(BF16)
            contrib = _dot(ctx, wo_h)
            rows = pl.ds(qi * BQ, BQ)
            if first is False:
                acc_v[rows, :] += contrib
            else:
                acc_v[rows, :] = contrib + jnp.where(first, 0.0, acc_v[rows, :])

        fq = list(fillers_qk)
        fh = list(fillers_head)
        tiles = [(i, t) for i in range(NQ) for t in range(i + 1)]
        qptr = [0]

        def emit_qk_upto(n):
            emitted = False
            while qptr[0] < min(n, len(tiles)):
                i, t = tiles[qptr[0]]
                qk(i, t)
                if fh:
                    fh.pop(0)()
                if t == i:
                    fin_max(i)
                qptr[0] += 1
                emitted = True
            return emitted

        def T(i):
            return i * (i + 1) // 2

        emit_qk_upto(1)
        for (qi, t) in tiles:
            need = T(qi + 2) if t == qi else T(qi + 1) + t + 1
            pv(qi, t)
            if not emit_qk_upto(need) and qptr[0] >= len(tiles) and fq:
                fq.pop(0)()
            if t == qi:
                fin(qi)
        _run(fq)
        _run(fillers_v)

    def vhead(hd):
        return [P(proj_v, hd, r, PCH) for r in range(S - ROT, S, PCH)]

    def head_body(hd, _):
        fq = [P(proj_q, hd + 1, r, PCH) for r in range(0, S, PCH)]
        fk = [P(proj_k, hd + 1, r, PCH) for r in range(0, S, PCH)]
        fv = [P(proj_v, hd + 1, r, PCH) for r in range(0, S - ROT, PCH)]
        attention(hd, False, fq + fk, fv, vhead(hd), k_v, v_v)
        return 0

    def first_body(hd, _):
        fq = [P(proj_q, hd + 1, r, 256) for r in range(0, S - QROT, 256)]
        fhq = [P(proj_q, hd, r, 256) for r in range(S - QROT, S, 256)]
        attention(hd, hd == 0, fq, [], fhq, k_pre.at[hd], v_pre.at[hd])
        return 0

    lax.fori_loop(0, LA - 1, first_body, 0)
    for r in range(S - QROT, S, 512):
        proj_q(LA - 1, r, 512)
    d_wo1.wait()
    go(*[f(g) for g in range(1, NG) for f in (d_uk, d_uv, d_q)], d_mb, *d_w)

    def group_body(g, _):
        @pl.when(g > 0)
        def _():
            d_uk(g).wait()
            d_uv(g).wait()
            d_q(g).wait()
            extract(wuk_r, g, wk_s, C)
            extract(wuv_r, g, wv_s, C)
            extract(wq_r, g, wq_s, M)
        lo = jnp.maximum(G * g - 1, LA - 1)
        hi = jnp.minimum(G * g + G - 1, H - 1)
        lax.fori_loop(lo, hi, head_body, 0)
        return 0

    lax.fori_loop(0, NG, group_body, 0)
    d_mb.wait()
    for d in d_w:
        d.wait()
    mod_v[:, 2 * M:] = _dot(sc8, wmb_v[...])

    g_v[pl.ds(0, G0), :] = jnp.zeros((G0, M), F32)
    g_v[pl.ds(S + G0, G0), :] = jnp.zeros((G0, M), F32)
    outs = []
    c128 = lax.broadcasted_iota(jnp.int32, (RC, 128), 1)
    stB = {}

    def stA(r):
        rows = pl.ds(r * RC, RC)
        x1 = x_v[rows, :].astype(F32) + modrow(2) * acc_v[rows, :]
        acc_v[rows, :] = x1
        h2 = _ln(x1) * (1.0 + modrow(4)) + modrow(3)
        h_v[rows, :] = h2.astype(BF16)
        stB[r, 'lnh'] = _ln(h2).astype(BF16)

    def stB1(r):
        g = _gelu(_dot(stB.pop((r, 'lnh')), w1_v[...]))
        g_v[pl.ds(r * RC + G0, RC), :] = g

    def stC(r):
        base = r * RC + G0

        def sh(d, lo):
            return g_v[pl.ds(base + d, RC), lo:lo + 128]
        t0 = sh(-1, 0)
        t1 = jnp.where(c128 < 32, sh(-1, 128), sh(1, 128))
        t2 = jnp.where(c128 < 64, sh(1, 256), sh(-2, 256))
        t3 = jnp.where(c128 < 96, sh(-2, 384), sh(2, 384))
        t4 = sh(2, 512)
        gs = jnp.concatenate([t0, t1, t2, t3, t4], axis=1).astype(BF16)
        rows = pl.ds(r * RC, RC)
        stB[r, 'x1b'] = h_v[rows, :].astype(F32) + _dot(gs, w2_v[...])

    def stD(r):
        stB[r, 'ln'] = _ln(stB[r, 'x1b']).astype(BF16)

    def stE(r):
        stB[r, 'u'] = _gelu(_dot_nt(stB.pop((r, 'ln')), w3_v[...])).astype(BF16)

    def stF(r):
        rows = pl.ds(r * RC, RC)
        y = stB.pop((r, 'x1b')) + _dot(stB.pop((r, 'u')), w4_v[...])
        o_v[rows, :] = (acc_v[rows, :] + modrow(5) * y).astype(BF16)
        oc = pltpu.make_async_copy(o_v.at[rows, :], o_hbm.at[rows, :], sems.at[SEM_O + r])
        oc.start()
        outs.append(oc)

    seq = [('A', 0), ('B', 0), ('A', 1)]
    for r in range(NR + 1):
        seq += [('B', r + 1), ('C', r), ('D', r), ('F', r - 1), ('A', r + 2), ('E', r)]
    fnmap = dict(A=stA, B=stB1, C=stC, D=stD, E=stE, F=stF)
    bjobs = [P(fnmap[k], r) for k, r in seq if 0 <= r < NR]
    attention(H - 1, False, bjobs, [], vhead(H - 1), k_v, v_v)
    for oc in outs:
        oc.wait()


@jax.jit
def pallas_adaLN_cond__compressed_kv_cla__mixer_s_mlp__prompt_kernel(
    A_x: jax.Array,
    A_c_kv: jax.Array,
    A_w_q: jax.Array,
    A_w_uk: jax.Array,
    A_w_uv: jax.Array,
    A_w_o: jax.Array,
    B_x: jax.Array,
    B_w1: jax.Array,
    B_w2: jax.Array,
    B_w3: jax.Array,
    B_w4: jax.Array,
    c: jax.Array,
    w_mod: jax.Array,
):
    del B_x
    hbm = pl.BlockSpec(memory_space=pltpu.HBM)
    out = pl.pallas_call(
        _kernel,
        out_shape=jax.ShapeDtypeStruct((S, M), BF16),
        in_specs=[hbm] * 12 + [pl.BlockSpec(memory_space=pltpu.SMEM)],
        out_specs=hbm,
        scratch_shapes=[
            pltpu.VMEM((S, M), BF16), pltpu.VMEM((S, C), BF16),
            pltpu.VMEM((NG, M // 2, 8, D), U32), pltpu.VMEM((NG, C // 2, 8, D), U32),
            pltpu.VMEM((NG, C // 2, 8, D), U32),
            pltpu.VMEM((H, D, M), BF16),
            pltpu.VMEM((M, M), BF16), pltpu.VMEM((M, M), BF16), pltpu.VMEM((F, M), BF16), pltpu.VMEM((F, M), BF16),
            pltpu.VMEM((1, M), BF16), pltpu.VMEM((M, 2 * M), BF16), pltpu.VMEM((M, 4 * M), BF16),
            pltpu.VMEM((H, M, D), BF16), pltpu.VMEM((H, C, D), BF16), pltpu.VMEM((H, C, D), BF16),
            pltpu.VMEM((8, 6 * M), F32),
            pltpu.VMEM((S, M), BF16),
            pltpu.VMEM((S, D), BF16), pltpu.VMEM((S, D), BF16), pltpu.VMEM((S, D), BF16),
            pltpu.VMEM((LA - 1, S, D), BF16), pltpu.VMEM((LA - 1, S, D), BF16),
            pltpu.VMEM((S, M), F32),
            pltpu.VMEM((S + 2 * G0, M), F32),
            pltpu.VMEM((S, M), BF16),
            pltpu.SemaphoreType.DMA((56,)),
        ],
        compiler_params=pltpu.CompilerParams(vmem_limit_bytes=110 * 1024 * 1024),
    )(A_x.reshape(S, M), A_c_kv.reshape(S, C),
      A_w_q.reshape(M // 2, 2, H, D), A_w_uk.reshape(C // 2, 2, H, D), A_w_uv.reshape(C // 2, 2, H, D),
      A_w_o, B_w1, B_w2, B_w3.T, B_w4, c, w_mod, np.zeros((1,), np.int32))
    return out.reshape(1, S, M)
```

```python
import functools

import jax
import jax.numpy as jnp
import numpy as np
from jax import lax
import jax.experimental.pallas as pl
import jax.experimental.pallas.tpu as pltpu

F32 = jnp.float32
BF16 = jnp.bfloat16
U32 = jnp.uint32
LOG2E = 1.4426950408889634
NEG = -1e9 * LOG2E

S, M, C, H, D, F = 2048, 640, 512, 32, 128, 1728
BQ = 256
NQ = S // BQ
G = 8
NG = H // G
PG = G // 2
LA = 4
LAG = 2
ROT = 1536
QROT = 512
PCH = 512
RC = 256
NR = S // RC
G0 = 8


def _dot(a, b):
    return jnp.dot(a, b, preferred_element_type=F32)


def _dot_nt(a, b):
    return lax.dot_general(a, b, (((1,), (1,)), ((), ())), preferred_element_type=F32)


def _ln(x):
    m = jnp.mean(x, axis=-1, keepdims=True)
    xc = x - m
    v = jnp.mean(xc * xc, axis=-1, keepdims=True)
    return xc * lax.rsqrt(v + 1e-5)


def _gelu(x):
    return jax.nn.gelu(x, approximate=True)


class _Multi:
    def __init__(self, ds):
        self.ds = ds

    def start(self):
        for d in self.ds:
            d.start()

    def wait(self):
        for d in self.ds:
            d.wait()


def _interleave(a, b):
    na, nb = len(a), len(b)
    ia = ib = 0
    out = []
    while ia < na or ib < nb:
        if ib >= nb or (ia < na and ia * max(nb, 1) <= ib * max(na, 1)):
            out.append(a[ia])
            ia += 1
        else:
            out.append(b[ib])
            ib += 1
    return out


def _run(jobs):
    for f in jobs:
        f()


def _kernel(x_hbm, ckv_hbm, wq_hbm, wuk_hbm, wuv_hbm, wo_hbm, w1_hbm, w2_hbm, w3_hbm, w4_hbm, c_hbm, wmod_hbm,
            zero_ref, o_hbm,
            x_v, ckv_v, wq_r, wuk_r, wuv_r, wo_v, w1_v, w2_v, w3_v, w4_v, c_v, wma_v, wmb_v,
            wq_s, wk_s, wv_s, mod_v, h_v, q_v, k_v, v_v, k_pre, v_pre, acc_v, g_v, o_v, sems):
    P = functools.partial

    def cp(i, src, dst):
        return pltpu.make_async_copy(src, dst, sems.at[i])

    def wcp(i, hbm, raw, g):
        hu = hbm.bitcast(U32)
        return _Multi([cp(i + 2 * g + e, hu.at[:, e, pl.ds(PG * g, PG), :], raw.at[g, :, pl.ds(PG * e, PG), :])
                       for e in range(2)])

    NW = LA - 1
    d_ckv = cp(0, ckv_hbm, ckv_v)
    d_uk = lambda g: wcp(32, wuk_hbm, wuk_r, g)
    d_uv = lambda g: wcp(40, wuv_hbm, wuv_r, g)
    d_q = lambda g: wcp(48, wq_hbm, wq_r, g)
    d_c = cp(7, c_hbm, c_v)
    d_ma = cp(8, wmod_hbm.at[:, pl.ds(0, 2 * M)], wma_v)
    d_mb = cp(9, wmod_hbm.at[:, pl.ds(2 * M, 4 * M)], wmb_v)
    d_x = cp(10, x_hbm, x_v)
    d_wo0 = cp(11, wo_hbm.at[pl.ds(0, NW)], wo_v.at[pl.ds(0, NW)])
    d_wo1 = cp(12, wo_hbm.at[pl.ds(NW, H - NW)], wo_v.at[pl.ds(NW, H - NW)])
    d_w = [cp(13, w1_hbm, w1_v), cp(14, w2_hbm, w2_v), cp(15, w3_hbm, w3_v), cp(16, w4_hbm, w4_v)]
    SEM_O = 17

    def go(*ds):
        for d in ds:
            d.start()

    def extract_pair(raw, g, dst, n, j):
        r2 = raw.at[g].reshape(n * PG, D)
        b = r2[pl.ds(j, n, stride=PG), :]
        dst[G * g + 2 * j] = pltpu.bitcast(b << U32(16), F32).astype(BF16)
        dst[G * g + 2 * j + 1] = pltpu.bitcast(b & U32(0xFFFF0000), F32).astype(BF16)

    def extract(raw, g, dst, n):
        for j in range(PG):
            extract_pair(raw, g, dst, n, j)

    qscale = (D ** -0.5) * LOG2E

    def proj_q(hd, r, n):
        rows = pl.ds(r, n)
        q_v[rows, :] = (_dot(h_v[rows, :], wq_s[hd]) * qscale).astype(BF16)

    def proj_k(hd, r, n, dst=None):
        rows = pl.ds(r, n)
        dst = k_v if dst is None else dst
        dst[rows, :] = _dot(ckv_v[rows, :], wk_s[hd]).astype(BF16)

    def proj_v(hd, r, n, dst=None):
        rows = pl.ds(r, n)
        dst = v_v if dst is None else dst
        dst[rows, :] = _dot(ckv_v[rows, :], wv_s[hd]).astype(BF16)

    def modrow(i):
        return mod_v[0:1, i * M:(i + 1) * M]

    def ln_rows(r, n):
        rows = pl.ds(r, n)
        xx = x_v[rows, :].astype(F32)
        h_v[rows, :] = (_ln(xx) * (1.0 + modrow(1)) + modrow(0)).astype(BF16)

    def kdst(hd):
        return k_v if hd == LA - 1 else k_pre.at[hd]

    def vdst(hd):
        return v_v if hd == LA - 1 else v_pre.at[hd]

    def zip_first(ex, jobs):
        out = []
        exi = 0
        for n, f in enumerate(jobs):
            need = min((n // 8) // 2 + 1, PG)
            want = max(need, min(PG, n + 1))
            while exi < want:
                out.append(ex[exi])
                exi += 1
            out.append(f)
        return out + ex[exi:]

    kjobs = [P(proj_k, hd, r, 256, kdst(hd)) for hd in range(LA) for r in range(0, S, 256)]
    qjobs = [P(proj_q, 0, r, 256) for r in range(0, S - QROT, 256)]
    exk = [P(extract_pair, wuk_r, 0, wk_s, C, j) for j in range(PG)]
    exv = [P(extract_pair, wuv_r, 0, wv_s, C, j) for j in range(PG)]
    exq = [P(extract_pair, wq_r, 0, wq_s, M, j) for j in range(PG)]

    go(d_uk(0), d_ckv)
    d_uk(0).wait()
    kz = zip_first(exk, kjobs)
    for n, f in enumerate(kz):
        if n == 1:
            d_ckv.wait()
            go(d_uv(0), d_c, d_ma, d_x)
        if n == 6:
            go(d_q(0), d_wo0)
        if n == len(kz) - 4:
            d_uv(0).wait()
            _run(_interleave(kz[n:], exv))
            break
        f()
    _run([P(proj_v, 0, r, 256, vdst(0)) for r in range(0, S, 256)])
    d_c.wait()
    d_ma.wait()
    d_x.wait()
    cc = c_v[...].astype(F32)
    sc8 = jnp.broadcast_to((cc * jax.nn.sigmoid(cc)).astype(BF16), (8, M))
    mod_v[:, 0:2 * M] = _dot(sc8, wma_v[...])
    NI, LNC = 2, 64

    def v_ln(i, _):
        r0 = pl.multiple_of(i * (S // NI), S // NI)
        r1 = pl.multiple_of(i * ((S - ROT) // NI), 128)
        jobs = [P(proj_v, hd, r0 + r, 256, vdst(hd)) for hd in range(1, LA - 1) for r in range(0, S // NI, 256)]
        jobs.append(P(proj_v, LA - 1, r1, (S - ROT) // NI, vdst(LA - 1)))
        _run(_interleave(jobs, [P(ln_rows, r0 + k * LNC, LNC) for k in range((S // NI) // LNC)]))
        return 0

    lax.fori_loop(0, NI, v_ln, 0)
    d_q(0).wait()
    go(d_wo1)
    _run(zip_first(exq, qjobs))
    d_wo0.wait()

    never = lax.broadcasted_iota(jnp.int32, (BQ, 128), 1) < zero_ref[0]
    tri = lax.broadcasted_iota(jnp.int32, (128, 128), 1) <= lax.broadcasted_iota(jnp.int32, (128, 128), 0)

    def attention(hd, first, fillers_qk, fillers_v, fillers_head, k_ref, v_ref):
        wo_h = wo_v[hd]
        st = {}
        hist = []

        def qk(qi, t):
            d = st.setdefault(qi, dict(ss={}, mp=None, lp=None, acc=None))
            q = q_v[pl.ds(qi * BQ, BQ), :]
            if t < qi:
                s = _dot_nt(q, k_ref[pl.ds(t * 256, 256), :])
                d['ss'][t] = s
                x = jnp.maximum(s[:, :128], s[:, 128:])
            else:
                s0 = _dot_nt(q, k_ref[pl.ds(t * 256, 128), :])
                s1 = _dot_nt(q[128:], k_ref[pl.ds(t * 256 + 128, 128), :])
                s0 = jnp.concatenate([jnp.where(tri, s0[:128], NEG), s0[128:]], axis=0)
                s1 = jnp.where(tri, s1, NEG)
                d['ss'][t] = (s0, s1)
                x = jnp.concatenate([s0[:128], jnp.maximum(s0[128:], s1)], axis=0)
            d['mp'] = x if d['mp'] is None else jnp.maximum(d['mp'], x)

        def fin_max(qi):
            m = jnp.max(st[qi]['mp'], axis=-1, keepdims=True)
            st[qi]['m'] = jnp.broadcast_to(m, (BQ, 128))

        def pv(qi, t):
            d = st[qi]
            mm = d['m']
            if len(hist) >= LAG:
                mm = jnp.where(never, hist[-LAG], mm)
            if t < qi:
                p = jnp.exp2(d['ss'][t] - jnp.concatenate([mm, mm], axis=1))
                o = _dot(p.astype(BF16), v_ref[pl.ds(t * 256, 256), :])
                x = p[:, :128] + p[:, 128:]
            else:
                s0, s1 = d['ss'][t]
                p0 = jnp.exp2(s0 - mm)
                p1 = jnp.exp2(s1 - mm[128:])
                o0 = _dot(p0.astype(BF16), v_ref[pl.ds(t * 256, 128), :])
                o1 = _dot(p1.astype(BF16), v_ref[pl.ds(t * 256 + 128, 128), :])
                o = jnp.concatenate([o0[:128], o0[128:] + o1], axis=0)
                x = jnp.concatenate([p0[:128], p0[128:] + p1], axis=0)
            hist.append(o)
            d['lp'] = x if d['lp'] is None else d['lp'] + x
            d['acc'] = o if d['acc'] is None else d['acc'] + o

        def fin(qi):
            d = st.pop(qi)
            l = jnp.sum(d['lp'], axis=-1, keepdims=True)
            ctx = (d['acc'] / l).astype(BF16)
            contrib = _dot(ctx, wo_h)
            rows = pl.ds(qi * BQ, BQ)
            if first is False:
                acc_v[rows, :] += contrib
            else:
                acc_v[rows, :] = contrib + jnp.where(first, 0.0, acc_v[rows, :])

        fq = list(fillers_qk)
        fh = list(fillers_head)
        tiles = [(i, t) for i in range(NQ) for t in range(i + 1)]
        qptr = [0]

        def emit_qk_upto(n):
            emitted = False
            while qptr[0] < min(n, len(tiles)):
                i, t = tiles[qptr[0]]
                qk(i, t)
                if fh:
                    fh.pop(0)()
                if t == i:
                    fin_max(i)
                qptr[0] += 1
                emitted = True
            return emitted

        def T(i):
            return i * (i + 1) // 2

        emit_qk_upto(1)
        for (qi, t) in tiles:
            need = T(qi + 2) if t == qi else T(qi + 1) + t + 1
            pv(qi, t)
            if not emit_qk_upto(need) and qptr[0] >= len(tiles) and fq:
                fq.pop(0)()
            if t == qi:
                if qi == NQ - 1 and fq:
                    fq.pop(0)()
                fin(qi)
        _run(fq)
        _run(fillers_v)

    def vhead(hd):
        return [P(proj_v, hd, r, PCH) for r in range(S - ROT, S, PCH)]

    def head_body(hd, _):
        fq = [P(proj_q, hd + 1, r, PCH) for r in range(0, S, PCH)]
        fk = [P(proj_k, hd + 1, r, PCH) for r in range(0, S, PCH)]
        fv = [P(proj_v, hd + 1, r, PCH) for r in range(0, S - ROT, PCH)]
        attention(hd, False, fk + fq, fv, vhead(hd), k_v, v_v)
        return 0

    def first_body(hd, _):
        fq = [P(proj_q, hd + 1, r, 256) for r in range(0, S - QROT, 256)]
        fhq = [P(proj_q, hd, r, 256) for r in range(S - QROT, S, 256)]
        attention(hd, hd == 0, fq, [], fhq, k_pre.at[hd], v_pre.at[hd])
        return 0

    lax.fori_loop(0, LA - 1, first_body, 0)
    for r in range(S - QROT, S, 512):
        proj_q(LA - 1, r, 512)
    d_wo1.wait()
    go(*[f(g) for g in range(1, NG) for f in (d_uk, d_uv, d_q)], d_mb, *d_w)

    def group_body(g, _):
        @pl.when(g > 0)
        def _():
            d_uk(g).wait()
            d_uv(g).wait()
            d_q(g).wait()
            extract(wuk_r, g, wk_s, C)
            extract(wuv_r, g, wv_s, C)
            extract(wq_r, g, wq_s, M)
        lo = jnp.maximum(G * g - 1, LA - 1)
        hi = jnp.minimum(G * g + G - 1, H - 1)

        assert LA % 2 == 0 and G % 2 == 0 and H % G == 0

        def two_heads(i, _):
            head_body(lo + 2 * i, 0)
            head_body(lo + 2 * i + 1, 0)
            return 0
        lax.fori_loop(0, (hi - lo) // 2, two_heads, 0)
        return 0

    lax.fori_loop(0, NG, group_body, 0)
    d_mb.wait()
    for d in d_w:
        d.wait()
    mod_v[:, 2 * M:] = _dot(sc8, wmb_v[...])

    g_v[pl.ds(0, G0), :] = jnp.zeros((G0, M), F32)
    g_v[pl.ds(S + G0, G0), :] = jnp.zeros((G0, M), F32)
    outs = []
    c128 = lax.broadcasted_iota(jnp.int32, (RC, 128), 1)
    stB = {}

    def stA(r):
        rows = pl.ds(r * RC, RC)
        x1 = x_v[rows, :].astype(F32) + modrow(2) * acc_v[rows, :]
        acc_v[rows, :] = x1
        h2 = _ln(x1) * (1.0 + modrow(4)) + modrow(3)
        h_v[rows, :] = h2.astype(BF16)
        stB[r, 'lnh'] = _ln(h2).astype(BF16)

    def stB1(r):
        g = _gelu(_dot(stB.pop((r, 'lnh')), w1_v[...]))
        g_v[pl.ds(r * RC + G0, RC), :] = g

    def stC(r):
        base = r * RC + G0

        def sh(d, lo):
            return g_v[pl.ds(base + d, RC), lo:lo + 128]
        t0 = sh(-1, 0)
        t1 = jnp.where(c128 < 32, sh(-1, 128), sh(1, 128))
        t2 = jnp.where(c128 < 64, sh(1, 256), sh(-2, 256))
        t3 = jnp.where(c128 < 96, sh(-2, 384), sh(2, 384))
        t4 = sh(2, 512)
        gs = jnp.concatenate([t0, t1, t2, t3, t4], axis=1).astype(BF16)
        rows = pl.ds(r * RC, RC)
        stB[r, 'x1b'] = h_v[rows, :].astype(F32) + _dot(gs, w2_v[...])

    def stD(r):
        stB[r, 'ln'] = _ln(stB[r, 'x1b']).astype(BF16)

    def stE(r):
        stB[r, 'u'] = _gelu(_dot_nt(stB.pop((r, 'ln')), w3_v[...])).astype(BF16)

    def stF(r):
        rows = pl.ds(r * RC, RC)
        y = stB.pop((r, 'x1b')) + _dot(stB.pop((r, 'u')), w4_v[...])
        o_v[rows, :] = (acc_v[rows, :] + modrow(5) * y).astype(BF16)
        oc = pltpu.make_async_copy(o_v.at[rows, :], o_hbm.at[rows, :], sems.at[SEM_O + r])
        oc.start()
        outs.append(oc)

    seq = [('A', 0), ('B', 0), ('A', 1)]
    for r in range(NR + 1):
        seq += [('B', r + 1), ('C', r), ('D', r), ('F', r - 1), ('A', r + 2), ('E', r)]
    fnmap = dict(A=stA, B=stB1, C=stC, D=stD, E=stE, F=stF)
    bjobs = [P(fnmap[k], r) for k, r in seq if 0 <= r < NR]
    attention(H - 1, False, bjobs, [], vhead(H - 1), k_v, v_v)
    for oc in outs:
        oc.wait()


@jax.jit
def pallas_adaLN_cond__compressed_kv_cla__mixer_s_mlp__prompt_kernel(
    A_x: jax.Array,
    A_c_kv: jax.Array,
    A_w_q: jax.Array,
    A_w_uk: jax.Array,
    A_w_uv: jax.Array,
    A_w_o: jax.Array,
    B_x: jax.Array,
    B_w1: jax.Array,
    B_w2: jax.Array,
    B_w3: jax.Array,
    B_w4: jax.Array,
    c: jax.Array,
    w_mod: jax.Array,
):
    del B_x
    hbm = pl.BlockSpec(memory_space=pltpu.HBM)
    out = pl.pallas_call(
        _kernel,
        out_shape=jax.ShapeDtypeStruct((S, M), BF16),
        in_specs=[hbm] * 12 + [pl.BlockSpec(memory_space=pltpu.SMEM)],
        out_specs=hbm,
        scratch_shapes=[
            pltpu.VMEM((S, M), BF16), pltpu.VMEM((S, C), BF16),
            pltpu.VMEM((NG, M // 2, 8, D), U32), pltpu.VMEM((NG, C // 2, 8, D), U32),
            pltpu.VMEM((NG, C // 2, 8, D), U32),
            pltpu.VMEM((H, D, M), BF16),
            pltpu.VMEM((M, M), BF16), pltpu.VMEM((M, M), BF16), pltpu.VMEM((F, M), BF16), pltpu.VMEM((F, M), BF16),
            pltpu.VMEM((1, M), BF16), pltpu.VMEM((M, 2 * M), BF16), pltpu.VMEM((M, 4 * M), BF16),
            pltpu.VMEM((H, M, D), BF16), pltpu.VMEM((H, C, D), BF16), pltpu.VMEM((H, C, D), BF16),
            pltpu.VMEM((8, 6 * M), F32),
            pltpu.VMEM((S, M), BF16),
            pltpu.VMEM((S, D), BF16), pltpu.VMEM((S, D), BF16), pltpu.VMEM((S, D), BF16),
            pltpu.VMEM((LA - 1, S, D), BF16), pltpu.VMEM((LA - 1, S, D), BF16),
            pltpu.VMEM((S, M), F32),
            pltpu.VMEM((S + 2 * G0, M), F32),
            pltpu.VMEM((S, M), BF16),
            pltpu.SemaphoreType.DMA((56,)),
        ],
        compiler_params=pltpu.CompilerParams(vmem_limit_bytes=110 * 1024 * 1024),
    )(A_x.reshape(S, M), A_c_kv.reshape(S, C),
      A_w_q.reshape(M // 2, 2, H, D), A_w_uk.reshape(C // 2, 2, H, D), A_w_uv.reshape(C // 2, 2, H, D),
      A_w_o, B_w1, B_w2, B_w3.T, B_w4, c, w_mod, np.zeros((1,), np.int32))
    return out.reshape(1, S, M)
```
